```python
import os as _os
_os.environ.setdefault("JAX_PLATFORMS", "cpu")
import jax
import jax.numpy as jnp

def _softmax(x, axis=-1):
    return jax.nn.softmax(x, axis=axis)
def _gelu(x):
    return jax.nn.gelu(x, approximate=True)
def _silu(x):
    return jax.nn.silu(x)
def _sigmoid(x):
    return jax.nn.sigmoid(x)
def _layernorm(x, axis=-1, eps=1e-5):
    m = jnp.mean(x, axis=axis, keepdims=True)
    v = jnp.var(x, axis=axis, keepdims=True)
    return (x - m) / jnp.sqrt(v + eps)
def _scatter_add(tgt, idx, src, axis=0):
    return tgt.at[idx].add(src)
def _segment_sum(src, seg, n):
    return jax.ops.segment_sum(src, seg, n)
class _Rng:
    def __init__(self, key):
        self._k = key
    def _next(self):
        self._k, sub = jax.random.split(self._k)
        return sub
    def normal(self, shape):
        return jax.random.normal(self._next(), shape, dtype=jnp.bfloat16)
    def randint(self, lo, hi, shape):
        return jax.random.randint(self._next(), shape, lo, hi, dtype=jnp.int32)
    def uniform(self, shape, lo=0.0, hi=1.0):
        return jax.random.uniform(self._next(), shape, jnp.bfloat16, lo, hi)
    def permutation(self, n):
        return jax.random.permutation(self._next(), n)


kernel_name = 'parallel_sum__sliding_block_cached__dense_activation_mish__decode'

def setup_inputs():
    _rng = _Rng(jax.random.key(int.from_bytes(__import__("os").urandom(4), "little")))
    _w = (lambda a: (lambda t: t.astype(jnp.bfloat16) if jnp.issubdtype(t.dtype, jnp.floating) else t)(jnp.asarray(a)))
    def _A_setup():
        B, Sq, D = 2, 1, 512
        Hq, Hkv, Sk, Dh = 32, 8, 32768, 128
        assert Hq % Hkv == 0, (Hq, Hkv)
        return {
            "x": _w((lambda *s: _rng.normal(s) * 0.05)(B, Sq, D)),
            "k_cache": _w((lambda *s: _rng.normal(s) * 0.8)(B, Hkv, Sk, Dh)),
            "v_cache": _w((lambda *s: _rng.normal(s) * 0.8)(B, Hkv, Sk, Dh)),
            "wq": _w((lambda *s: _rng.normal(s) * 0.8)(D, Hq * Dh) * (D ** -0.5)),
            "wo": _w((lambda *s: _rng.normal(s) * 0.8)(Hq * Dh, D) * ((Hq * Dh) ** -0.5)),
        }
    _A_in = _A_setup()

    def _B_setup():
        B, S, D, F = 2, 1, 512, 1792
        return {
            "x": _w((lambda *s: _rng.normal(s) * 0.05)(B, S, D)),
            "w1": _w((lambda *s: _rng.normal(s) * 0.4)(D, F) * (D ** -0.5)),
            "b1": _w((lambda *s: _rng.normal(s) * 0.05)(F)),
            "w2": _w((lambda *s: _rng.normal(s) * 0.05)(F, D) * (F ** -0.5)),
        }
    _B_in = _B_setup()

    return {
        "A_x": _A_in["x"],
        "A_k_cache": _A_in["k_cache"],
        "A_v_cache": _A_in["v_cache"],
        "A_wq": _A_in["wq"],
        "A_wo": _A_in["wo"],
        "B_x": _B_in["x"],
        "B_w1": _B_in["w1"],
        "B_b1": _B_in["b1"],
        "B_w2": _B_in["w2"],
    }

def reference(A_x, A_k_cache, A_v_cache, A_wq, A_wo, B_x, B_w1, B_b1, B_w2):
    def _A_ref(x, k_cache, v_cache, wq, wo):
        B, Sq, D = x.shape
        Hq, Dh = 32, 128
        Hkv, Sk = k_cache.shape[1], k_cache.shape[2]
        W = min(4096, max(256, Sk // 4))
        rep = Hq // Hkv
        q = (lambda x, *d: x.transpose(*d))((x @ wq).reshape(B, Sq, Hq, Dh), 0, 2, 1, 3)
        k = jnp.repeat(k_cache[:, :, Sk - W:, :], rep, axis=1)
        v = jnp.repeat(v_cache[:, :, Sk - W:, :], rep, axis=1)
        scores = jnp.einsum("bhqd,bhkd->bhqk", q, k) * (Dh ** -0.5)
        p = _softmax(scores, axis=-1)
        o = jnp.einsum("bhqk,bhkd->bhqd", p, v)
        return (lambda x, *d: x.transpose(*d))(o, 0, 2, 1, 3).reshape(B, Sq, Hq * Dh) @ wo

    def _B_ref(x, w1, b1, w2):
        h = jnp.einsum("bsd,df->bsf", x, w1) + b1
        sp = jnp.log1p(jnp.exp(-jnp.abs(h))) + jnp.where(h > 0, h, jnp.zeros_like(h))
        act = h * jnp.tanh(sp)
        return jnp.einsum("bsf,fd->bsd", act, w2)

    x = A_x
    xn = _layernorm(x, axis=-1)
    return x + _A_ref(xn, A_k_cache, A_v_cache, A_wq, A_wo) + _B_ref(xn, B_w1, B_b1, B_w2)
```

```python
import functools
import jax
import jax.numpy as jnp
from jax import lax
import jax.experimental.pallas as pl
import jax.experimental.pallas.tpu as pltpu

B, D = 2, 512
HQ, HKV, DH = 32, 8, 128
REP = HQ // HKV
F = 1792

def _kernel(x_hbm, k_hbm, v_hbm, wq_hbm, wo_hbm, w1_hbm, b1_hbm, w2_hbm, o_ref,
            x_buf, b1_buf, kbuf, vbuf, wq_buf, wo_buf, w1_buf, w2_buf, sems, *, W, SK):
    f32, bf16 = jnp.float32, jnp.bfloat16
    cp = pltpu.make_async_copy
    c_x = cp(x_hbm, x_buf, sems.at[0])
    c_b1 = cp(b1_hbm, b1_buf, sems.at[1])
    c_wq = cp(wq_hbm, wq_buf, sems.at[2])
    c_w1 = cp(w1_hbm, w1_buf, sems.at[3])
    c_w2 = cp(w2_hbm, w2_buf, sems.at[4])
    c_wo = [cp(wo_hbm.at[pl.ds(h * REP * DH, REP * DH), :], wo_buf.at[pl.ds(h * REP * DH, REP * DH), :], sems.at[5 + h]) for h in range(HKV)]
    c_k = [cp(k_hbm.at[:, h, pl.ds(SK - W, W), :], kbuf.at[h], sems.at[13 + h]) for h in range(HKV)]
    c_v = [cp(v_hbm.at[:, h, pl.ds(SK - W, W), :], vbuf.at[h], sems.at[21 + h]) for h in range(HKV)]

    c_wq.start()
    c_x.start()
    c_b1.start()
    for h in range(HKV):
        c_k[h].start()
        c_v[h].start()
    c_w1.start()
    c_w2.start()
    for h in range(HKV):
        c_wo[h].start()

    c_x.wait()
    row = lax.broadcasted_iota(jnp.int32, (8, D), 0)
    x2 = x_buf[...].astype(f32)
    x0 = x2[0:1]
    x1 = x2[1:2]
    x8 = jnp.where(row < REP, jnp.broadcast_to(x0, (8, D)), jnp.broadcast_to(x1, (8, D)))
    m = jnp.mean(x8, axis=-1, keepdims=True)
    xc = x8 - m
    var = jnp.mean(xc * xc, axis=-1, keepdims=True)
    xn = (xc / jnp.sqrt(var + 1e-5)).astype(bf16)

    c_wq.wait()
    qall = jnp.dot(xn, wq_buf[...], preferred_element_type=f32)
    row128 = lax.broadcasted_iota(jnp.int32, (8, DH), 0)
    g_of_row = row128 % REP
    top = row128 < REP
    scale = DH ** -0.5
    o_parts = []
    for h in range(HKV):
        qh = jnp.zeros((8, DH), f32)
        for g in range(REP):
            j = h * REP + g
            qh = jnp.where(g_of_row == g, qall[:, j * DH:(j + 1) * DH], qh)
        qh = qh.astype(bf16)
        c_k[h].wait()
        nt = (((1,), (1,)), ((), ()))
        s0 = lax.dot_general(qh, kbuf[h, 0], nt, preferred_element_type=f32)
        s1 = lax.dot_general(qh, kbuf[h, 1], nt, preferred_element_type=f32)
        roww = lax.broadcasted_iota(jnp.int32, (8, W), 0)
        s = jnp.where(roww < REP, s0, s1) * scale
        mx = jnp.max(s, axis=-1, keepdims=True)
        p = jnp.exp(s - mx)
        l = jnp.sum(p, axis=-1, keepdims=True)
        pb = p.astype(bf16)
        c_v[h].wait()
        o0 = jnp.dot(pb, vbuf[h, 0], preferred_element_type=f32)
        o1 = jnp.dot(pb, vbuf[h, 1], preferred_element_type=f32)
        oh = jnp.where(top, o0, o1) / l
        o_parts.append(jnp.concatenate([jnp.where(g_of_row == g, oh, 0.0) for g in range(REP)], axis=1).astype(bf16))

    c_w1.wait()
    c_b1.wait()
    b1v = b1_buf[...].astype(f32)
    b1row = jnp.concatenate([jnp.broadcast_to(b1v[r:r + 1], (8, DH)) for r in range(F // 128)], axis=1)
    hdn = jnp.dot(xn, w1_buf[...], preferred_element_type=f32) + b1row
    sp = jnp.log1p(jnp.exp(-jnp.abs(hdn))) + jnp.maximum(hdn, 0.0)
    act = (hdn * jnp.tanh(sp)).astype(bf16)
    c_w2.wait()
    mlp = jnp.dot(act, w2_buf[...], preferred_element_type=f32)

    acc = jnp.zeros((8, D), f32)
    for h in range(HKV):
        c_wo[h].wait()
        acc = acc + jnp.dot(o_parts[h], wo_buf[pl.ds(h * REP * DH, REP * DH), :], preferred_element_type=f32)
    a0 = jnp.sum(acc[0:REP], axis=0, keepdims=True)
    a1 = jnp.sum(acc[REP:2 * REP], axis=0, keepdims=True)
    r0 = x0 + a0 + mlp[0:1]
    r1 = x1 + a1 + mlp[REP:REP + 1]
    o_ref[...] = jnp.concatenate([r0, r1], axis=0).astype(o_ref.dtype)


@jax.jit
def pallas_parallel_sum__sliding_block_cached__dense_activation_mish__decode_kernel(
    A_x, A_k_cache, A_v_cache, A_wq, A_wo, B_x, B_w1, B_b1, B_w2,
):
    SK = A_k_cache.shape[2]
    W = min(4096, max(256, SK // 4))
    bf16 = jnp.bfloat16
    b1 = B_b1.reshape(F // 128, 128)
    x = A_x.reshape(B, D)
    any_spec = pl.BlockSpec(memory_space=pl.ANY)
    out = pl.pallas_call(
        functools.partial(_kernel, W=W, SK=SK),
        out_shape=jax.ShapeDtypeStruct((B, D), A_x.dtype),
        in_specs=[any_spec] * 8,
        out_specs=pl.BlockSpec(memory_space=pltpu.VMEM),
        scratch_shapes=[
            pltpu.VMEM((B, D), bf16),
            pltpu.VMEM((F // 128, 128), bf16),
            pltpu.VMEM((HKV, B, W, DH), bf16),
            pltpu.VMEM((HKV, B, W, DH), bf16),
            pltpu.VMEM((D, HQ * DH), bf16),
            pltpu.VMEM((HQ * DH, D), bf16),
            pltpu.VMEM((D, F), bf16),
            pltpu.VMEM((F, D), bf16),
            pltpu.SemaphoreType.DMA((29,)),
        ],
        compiler_params=pltpu.CompilerParams(vmem_limit_bytes=100 * 1024 * 1024, disable_semaphore_checks=True),
    )(x, A_k_cache, A_v_cache, A_wq, A_wo, B_w1, b1, B_w2)
    return out.reshape(A_x.shape)
```

```python
import functools
import jax
import jax.numpy as jnp
from jax import lax
import jax.experimental.pallas as pl
import jax.experimental.pallas.tpu as pltpu

B, D = 2, 512
HQ, HKV, DH = 32, 8, 128
REP = HQ // HKV
F = 1792
NBH = B * HKV
CK = 128
G = 512

CFG = dict(lead=22, lag=30, extra=14, extra2=12, wq_step=16, kvcyc=16, w1_step=16, w2_step=16, kv_shift=16, compute=True)


def _cyc(n, step):
    return [i for s in range(step) for i in range(s, n, step)]


def _kernel(x_hbm, k_hbm, v_hbm, wq_hbm, wo_hbm, w1_hbm, b1_hbm, w2_hbm, o_ref,
            x_buf, b1_buf, kbuf, vbuf, wq_buf, wo_buf, w1_buf, w2_buf,
            sems, *, W, SK, cfg):
    f32, bf16 = jnp.float32, jnp.bfloat16
    cp = pltpu.make_async_copy
    NG = W // G
    lead, lag = cfg["lead"], cfg["lag"]

    class _S:
        def __init__(self, base):
            self.base = base
        @property
        def at(self):
            return self
        def __getitem__(self, i):
            return sems.at[self.base + i]
    ksems, vsems, wosems = _S(5), _S(5 + NG), _S(5 + 2 * NG)

    def wq_c(i):
        r, c = (i // 2) * 8, (i % 2) * 2048
        return cp(wq_hbm.at[pl.ds(r, 8), pl.ds(c, 2048)], wq_buf.at[pl.ds(r, 8), pl.ds(c, 2048)], sems.at[2])

    def w1_c(i):
        return cp(w1_hbm.at[pl.ds(i * 8, 8), :], w1_buf.at[pl.ds(i * 8, 8), :], sems.at[3])

    def w2_c(i):
        return cp(w2_hbm.at[pl.ds(i * 32, 32), :], w2_buf.at[pl.ds(i * 32, 32), :], sems.at[4])

    sh = cfg["kv_shift"]

    def kv_c(src, dst, sem, j, c, r):
        off = j * G + c * CK
        if off == 0 and sh:
            return [cp(src.at[r, pl.ds(SK - W, CK - sh), :], dst.at[r, pl.ds(sh, CK - sh), :], sem.at[j]),
                    cp(src.at[r, pl.ds(SK - sh, sh), :], dst.at[r, pl.ds(0, sh), :], sem.at[j])]
        return [cp(src.at[r, pl.ds(SK - W + off - sh, CK), :], dst.at[r, pl.ds(off, CK), :], sem.at[j])]

    def wo_c(seg, g, r0, nr, si):
        return cp(wo_hbm.at[seg, g, pl.ds(r0, nr), :], wo_buf.at[seg, g, pl.ds(r0, nr), :], wosems.at[si])

    hi, lo = [], []
    hi += [[wq_c(i)] for i in _cyc(128, cfg["wq_step"])]
    p_k = len(hi)
    for j in range(NG):
        cl = cfg["kvcyc"]
        for r0 in range(0, NBH, cl):
            for c in range(G // CK):
                for r in range(r0, r0 + cl):
                    hi.append(kv_c(k_hbm, kbuf, ksems, j, c, r))
                    lo.append(kv_c(v_hbm, vbuf, vsems, j, c, r))
    lo += [[w1_c(i)] for i in _cyc(64, cfg["w1_step"])]
    lo += [[w2_c(i)] for i in _cyc(56, cfg["w2_step"])]
    wo_groups = []
    def add_cycle(stream, groups):
        blocks = []
        for grp in groups:
            blocks += [(seg, g, len(wo_groups)) for seg, g in grp]
            wo_groups.append(grp)
        for c in range(4):
            for seg, g, si in blocks:
                stream.append([wo_c(seg, g, c * 32, 32, si)])
    add_cycle(hi, [[(s_, 0) for s_ in range(8)]])
    add_cycle(hi, [[(s_, 1) for s_ in range(4)]])
    add_cycle(hi, [[(4, 1), (5, 1)]])
    add_cycle(lo, [[(s_, 2) for s_ in range(8)], [(6, 1), (7, 1)]])
    add_cycle(lo, [[(s_, 3) for s_ in range(4)]])
    add_cycle(lo, [[(4, 3), (5, 3)]])
    for seg in (6, 7):
        si = len(wo_groups)
        wo_groups.append([(seg, 3)])
        lo += [[wo_c(seg, 3, r, 8, si)] for r in range(0, 128, 8)]
    wo_regions = [[3, 4], [1, 5], [2, 6], [7], [8]]

    seq = [(c, 1) for u in lo[:lead] for c in u]
    pos_of_pair = []
    rest = lo[lead:]
    for i in range(max(len(hi), len(rest))):
        if i < len(hi):
            seq += [(c, 0) for c in hi[i]]
        if i < len(rest):
            seq += [(c, 1) for c in rest[i]]
        pos_of_pair.append(len(seq))
    issued = [0]

    def issue_until_pair(p):
        end = len(seq) if p is None or p >= len(pos_of_pair) else pos_of_pair[p]
        for c, pr in seq[issued[0]:end]:
            c.start(priority=pr)
        issued[0] = max(issued[0], end)

    c_x = cp(x_hbm, x_buf, sems.at[0])
    c_b1 = cp(b1_hbm, b1_buf, sems.at[1])
    seq[0][0].start(priority=seq[0][1])
    issued[0] = 1
    c_x.start(priority=0)
    c_b1.start(priority=0)
    issue_until_pair(p_k - 1 + lag)

    if not cfg["compute"]:
        issue_until_pair(None)
        c_x.wait(); c_b1.wait()
        for i, b in ((2, wq_buf), (3, w1_buf), (4, w2_buf)):
            cp(b, b, sems.at[i]).wait()
        for j in range(NG):
            kg = kbuf.at[:, pl.ds(j * G, G), :]
            cp(kg, kg, ksems.at[j]).wait()
            cp(kg, kg, vsems.at[j]).wait()
        for si, blocks in enumerate(wo_groups):
            ref = wo_buf.at[pl.ds(blocks[0][0], len(blocks)), blocks[0][1]]
            cp(ref, ref, wosems.at[si]).wait()
        o_ref[...] = x_buf[...]
        return

    c_x.wait()
    row = lax.broadcasted_iota(jnp.int32, (8, D), 0)
    x2 = x_buf[...].astype(f32)
    x8 = jnp.where(row % 2 == 0, jnp.broadcast_to(x2[0:1], (8, D)), jnp.broadcast_to(x2[1:2], (8, D)))
    mu = jnp.mean(x8, axis=-1, keepdims=True)
    xc = x8 - mu
    var = jnp.mean(xc * xc, axis=-1, keepdims=True)
    xn = (xc / jnp.sqrt(var + 1e-5)).astype(bf16)

    row128 = lax.broadcasted_iota(jnp.int32, (8, DH), 0)
    g_of_row = row128 // 2
    even = row128 % 2 == 0

    cp(wq_buf, wq_buf, sems.at[2]).wait()
    qall = jnp.dot(xn, wq_buf[...], preferred_element_type=f32)
    qs = []
    for h in range(HKV):
        qh = qall[:, h * REP * DH:(h * REP + 1) * DH]
        for g in range(1, REP):
            j = h * REP + g
            qh = jnp.where(g_of_row == g, qall[:, j * DH:(j + 1) * DH], qh)
        qs.append(qh.astype(bf16))

    issue_until_pair(p_k + 63 + lag)

    scale = DH ** -0.5
    nt = (((1,), (1,)), ((), ()))
    eveng = lax.broadcasted_iota(jnp.int32, (8, G), 0) % 2 == 0
    ms = [None] * HKV
    ls = [None] * HKV
    accs = [None] * HKV

    for j in range(NG):
        base = j * G
        kg = kbuf.at[:, pl.ds(base, G), :]
        vg = vbuf.at[:, pl.ds(base, G), :]
        cp(kg, kg, ksems.at[j]).wait()
        cp(vg, vg, vsems.at[j]).wait()
        if j < NG - 1:
            issue_until_pair(p_k + (j + 2) * 64 - 1 + lag)
        else:
            cp(w1_buf, w1_buf, sems.at[3]).wait()
            c_b1.wait()
            issue_until_pair(p_k + NG * 64 - 1 + lag + cfg["extra"])
        ss = []
        for h in range(HKV):
            s0 = lax.dot_general(qs[h], kbuf[h, pl.ds(base, G), :], nt, preferred_element_type=f32)
            s1 = lax.dot_general(qs[h], kbuf[HKV + h, pl.ds(base, G), :], nt, preferred_element_type=f32)
            ss.append(jnp.where(eveng, s0, s1) * scale)
        pbs, alphas = [], []
        for h in range(HKV):
            s = ss[h]
            m_cur = jnp.max(s, axis=-1, keepdims=True)
            m_new = m_cur if j == 0 else jnp.maximum(ms[h], m_cur)
            p = jnp.exp(s - m_new)
            psum = p[:, 0:DH]
            for t in range(1, G // DH):
                psum = psum + p[:, t * DH:(t + 1) * DH]
            if j == 0:
                alphas.append(None)
                ls[h] = psum
            else:
                alpha = jnp.exp(ms[h] - m_new)
                alphas.append(alpha)
                ls[h] = ls[h] * alpha + psum
            pbs.append(p.astype(bf16))
            ms[h] = m_new
        for h in range(HKV):
            o0 = jnp.dot(pbs[h], vbuf[h, pl.ds(base, G), :], preferred_element_type=f32)
            o1 = jnp.dot(pbs[h], vbuf[HKV + h, pl.ds(base, G), :], preferred_element_type=f32)
            o = jnp.where(even, o0, o1)
            accs[h] = o if j == 0 else accs[h] * alphas[h] + o

    lhs = {}
    for h in range(HKV):
        l = jnp.sum(ls[h], axis=-1, keepdims=True)
        oh = accs[h] / l
        for g in range(REP):
            og = oh if g == 0 else pltpu.roll(oh, 8 - 2 * g, 0)
            lhs[(h, g)] = og.astype(bf16)

    b1v = b1_buf[...].astype(f32)
    b1row = jnp.concatenate([jnp.broadcast_to(b1v[r:r + 1], (8, DH)) for r in range(F // 128)], axis=1)
    hdn = jnp.dot(xn, w1_buf[...], preferred_element_type=f32) + b1row
    sp = jnp.log1p(jnp.exp(-jnp.abs(hdn))) + jnp.maximum(hdn, 0.0)
    act = (hdn * jnp.tanh(sp)).astype(bf16)

    cp(w2_buf, w2_buf, sems.at[4]).wait()
    ref0 = wo_buf.at[:, 0]
    cp(ref0, ref0, wosems.at[0]).wait()
    issue_until_pair(p_k + NG * 64 - 1 + lag + cfg["extra"] + cfg["extra2"])
    out8 = x8 + jnp.dot(act, w2_buf[...], preferred_element_type=f32)
    for seg, g in wo_groups[0]:
        out8 = out8 + jnp.dot(lhs[(seg, g)], wo_buf[seg, g], preferred_element_type=f32)

    for region in wo_regions:
        for si in region:
            blocks = wo_groups[si]
            ref = wo_buf.at[pl.ds(blocks[0][0], len(blocks)), blocks[0][1]]
            cp(ref, ref, wosems.at[si]).wait()
        issue_until_pair(None)
        for si in region:
            for seg, g in wo_groups[si]:
                out8 = out8 + jnp.dot(lhs[(seg, g)], wo_buf[seg, g], preferred_element_type=f32)
    o_ref[...] = out8[0:B].astype(o_ref.dtype)


def build(**kw):
  cfg = dict(CFG, **kw)
  @jax.jit
  def kernel_fn(A_x, A_k_cache, A_v_cache, A_wq, A_wo, B_x, B_w1, B_b1, B_w2):
    SK = A_k_cache.shape[2]
    W = min(4096, max(256, SK // 4))
    bf16, f32 = jnp.bfloat16, jnp.float32
    b1 = B_b1.reshape(F // 128, 128)
    x = A_x.reshape(B, D)
    k = A_k_cache.reshape(NBH, SK, DH)
    v = A_v_cache.reshape(NBH, SK, DH)
    wo = A_wo.reshape(HKV, REP, DH, D)
    any_spec = pl.BlockSpec(memory_space=pl.ANY)
    out = pl.pallas_call(
        functools.partial(_kernel, W=W, SK=SK, cfg=cfg),
        out_shape=jax.ShapeDtypeStruct((B, D), A_x.dtype),
        in_specs=[any_spec] * 8,
        out_specs=pl.BlockSpec(memory_space=pltpu.VMEM),
        scratch_shapes=[
            pltpu.VMEM((B, D), bf16),
            pltpu.VMEM((F // 128, 128), bf16),
            pltpu.VMEM((NBH, W, DH), bf16),
            pltpu.VMEM((NBH, W, DH), bf16),
            pltpu.VMEM((D, HQ * DH), bf16),
            pltpu.VMEM((HKV, REP, DH, D), bf16),
            pltpu.VMEM((D, F), bf16),
            pltpu.VMEM((F, D), bf16),
            pltpu.SemaphoreType.DMA((5 + 2 * (W // G) + 10,)),
        ],
        compiler_params=pltpu.CompilerParams(vmem_limit_bytes=100 * 1024 * 1024, disable_semaphore_checks=True,
                                             disable_bounds_checks=True),
    )(x, k, v, A_wq, wo, B_w1, b1, B_w2)
    return out.reshape(A_x.shape)
  return kernel_fn

pallas_parallel_sum__sliding_block_cached__dense_activation_mish__decode_kernel = build(kv_shift=16)
```

```python
import functools

import jax
import jax.numpy as jnp
from jax import lax
import jax.experimental.pallas as pl
import jax.experimental.pallas.tpu as pltpu

B, D = 2, 512
HQ, HKV, DH = 32, 8, 128
REP = HQ // HKV
F = 1792
NBH = B * HKV
CK = 128
G = 512
UT = 16
STEP = 16

KV_SHIFT = 16
O_WQ, O_WO, O_W1, O_W2 = 2, 2, 1, 15

LEAD = 22
LAG = 30
EXTRA1, EXTRA2 = 14, 12
VSPLIT = (0, 10, 14, 16)
N_WO_GROUPS = 8


def _cyc(n, step):
    return [i for s in range(step) for i in range(s, n, step)]


def _tiles(w):
    r, c = w.shape
    return (w.reshape(r // 8, 8, c // 128, 128).transpose(0, 2, 1, 3)
            .reshape((r // 8) * (c // 128), 8, 128))


def _col_tiles(val, n_col_tiles):
    n = val.shape[0] // n_col_tiles
    v4 = val.reshape(n, n_col_tiles, 8, 128)
    return [v4[:, c].reshape(n * 8, 128) for c in range(n_col_tiles)]


def _kernel(x_hbm, k_hbm, v_hbm, wq_hbm, wo_hbm, w1_hbm, b1_hbm, w2_hbm, o_ref,
            x_buf, b1_buf, kbuf, vbuf, wq_buf, wo_buf, w1_buf, w2_buf, sems, *, W, SK):
    f32, bf16 = jnp.float32, jnp.bfloat16
    cp = pltpu.make_async_copy
    NG = W // G
    UPG = (G // CK) * NBH
    S_X, S_B1, S_WQ, S_W1, S_W2, S_K = 0, 1, 2, 3, 4, 5
    S_V = S_K + NG
    S_WO = S_V + NG
    S_LAST = S_WO + N_WO_GROUPS

    def w_units(src, dst, si, o):
        n = src.shape[0]

        def piece(a, m):
            return cp(src.at[pl.ds(a, m)], dst.at[pl.ds(a, m)], sems.at[si])

        def unit(u):
            if u == 0:
                return [piece(0, UT - o), piece(n - o, o)]
            return [piece(UT * u - o, UT)]
        return [unit(u) for u in _cyc(n // UT, STEP)]

    def kv_unit(src, dst, si, j, c, r):
        off, sh, sem = j * G + c * CK, KV_SHIFT, sems.at[si + j]
        if off == 0:
            return [cp(src.at[r, pl.ds(SK - W, CK - sh), :], dst.at[r, pl.ds(sh, CK - sh), :], sem),
                    cp(src.at[r, pl.ds(SK - sh, sh), :], dst.at[r, pl.ds(0, sh), :], sem)]
        return [cp(src.at[r, pl.ds(SK - W + off - sh, CK), :], dst.at[r, pl.ds(off, CK), :], sem)]

    def wo_unit(seg, g, t0, nt, si):
        a, sem = (seg * REP + g) * 64 + t0 - O_WO, sems.at[si]
        if a < 0:
            return [cp(wo_hbm.at[pl.ds(0, nt + a)], wo_buf.at[seg, g, pl.ds(t0 - a, nt + a)], sem),
                    cp(wo_hbm.at[pl.ds(wo_hbm.shape[0] + a, -a)], wo_buf.at[seg, g, pl.ds(t0, -a)], sem)]
        return [cp(wo_hbm.at[pl.ds(a, nt)], wo_buf.at[seg, g, pl.ds(t0, nt)], sem)]

    hi = w_units(wq_hbm, wq_buf, S_WQ, O_WQ)
    lo = []
    p_k = len(hi)
    for j in range(NG):
        for c in range(G // CK):
            for r in range(NBH):
                hi.append(kv_unit(k_hbm, kbuf, S_K, j, c, r))
                lo.append(kv_unit(v_hbm, vbuf, S_V, j, c, r))
    lo += w_units(w1_hbm, w1_buf, S_W1, O_W1)
    lo += w_units(w2_hbm, w2_buf, S_W2, O_W2)

    wo_groups = []

    def add_cycle(stream, groups):
        blocks = []
        for grp in groups:
            blocks += [(seg, g, S_WO + len(wo_groups)) for seg, g in grp]
            wo_groups.append(grp)
        for c in range(64 // UT):
            for seg, g, si in blocks:
                stream.append(wo_unit(seg, g, c * UT, UT, si))

    add_cycle(hi, [[(s, 0) for s in range(8)]])
    add_cycle(hi, [[(s, 1) for s in range(3)]])
    add_cycle(hi, [[(3, 1), (4, 1)]])
    add_cycle(lo, [[(s, 2) for s in range(8)], [(5, 1), (6, 1), (7, 1)]])
    add_cycle(lo, [[(s, 3) for s in range(4)]])
    add_cycle(lo, [[(4, 3), (5, 3)]])
    wo_groups.append([(6, 3)])
    lo += [wo_unit(6, 3, t, 4, S_WO + 7) for t in range(0, 64, 4)]
    for vi in range(len(VSPLIT) - 1):
        lo += [wo_unit(7, 3, 4 * a, 4, S_LAST + vi) for a in range(VSPLIT[vi], VSPLIT[vi + 1])]
    assert len(wo_groups) == N_WO_GROUPS
    wo_regions = [[3, 4], [1, 5], [2, 6], [7]]

    seq = [(c, 1) for u in lo[:LEAD] for c in u]
    pos_of_pair = []
    rest = lo[LEAD:]
    for i in range(max(len(hi), len(rest))):
        if i < len(hi):
            seq += [(c, 0) for c in hi[i]]
        if i < len(rest):
            seq += [(c, 1) for c in rest[i]]
        pos_of_pair.append(len(seq))
    issued = [0]

    def issue_until_pair(p):
        end = len(seq) if p is None or p >= len(pos_of_pair) else pos_of_pair[p]
        for c, pr in seq[issued[0]:end]:
            c.start(priority=pr)
        issued[0] = max(issued[0], end)

    def wait_all(ref, si):
        cp(ref, ref, sems.at[si]).wait()

    def wait_wo(gi):
        blocks = wo_groups[gi]
        wait_all(wo_buf.at[pl.ds(blocks[0][0], len(blocks)), blocks[0][1]], S_WO + gi)

    c_x = cp(x_hbm, x_buf, sems.at[S_X])
    c_b1 = cp(b1_hbm, b1_buf, sems.at[S_B1])
    seq[0][0].start(priority=seq[0][1])
    issued[0] = 1
    c_x.start(priority=0)
    c_b1.start(priority=0)
    issue_until_pair(p_k - 1 + LAG)

    c_x.wait()
    row = lax.broadcasted_iota(jnp.int32, (8, D), 0)
    x2 = x_buf[...].astype(f32)
    x8 = jnp.where(row % 2 == 0, jnp.broadcast_to(x2[0:1], (8, D)), jnp.broadcast_to(x2[1:2], (8, D)))
    mu = jnp.mean(x8, axis=-1, keepdims=True)
    xc = x8 - mu
    var = jnp.mean(xc * xc, axis=-1, keepdims=True)
    xn = (xc / jnp.sqrt(var + 1e-5)).astype(bf16)

    row128 = lax.broadcasted_iota(jnp.int32, (8, DH), 0)
    lane128 = lax.broadcasted_iota(jnp.int32, (8, DH), 1)
    g_of_row = row128 // 2
    even = row128 % 2 == 0

    wait_all(wq_buf, S_WQ)
    wq_cols = _col_tiles(wq_buf[...], HQ)
    qs = []
    for h in range(HKV):
        qh = None
        for g in range(REP):
            qg = jnp.dot(xn, wq_cols[h * REP + g], preferred_element_type=f32)
            qh = qg if g == 0 else jnp.where(g_of_row == g, qg, qh)
        qs.append(qh.astype(bf16))

    issue_until_pair(p_k + UPG - 1 + LAG)

    scale = DH ** -0.5
    nt = (((1,), (1,)), ((), ()))
    even_g = lax.broadcasted_iota(jnp.int32, (8, G), 0) % 2 == 0
    ms, ls, accs = [None] * HKV, [None] * HKV, [None] * HKV
    p_end = p_k + NG * UPG - 1 + LAG

    for j in range(NG):
        base = j * G
        wait_all(kbuf.at[:, pl.ds(base, G), :], S_K + j)
        wait_all(vbuf.at[:, pl.ds(base, G), :], S_V + j)
        if j < NG - 1:
            issue_until_pair(p_k + (j + 2) * UPG - 1 + LAG)
        else:
            issue_until_pair(p_end + EXTRA1)
            wait_all(w1_buf, S_W1)
            c_b1.wait()
        ss = []
        for h in range(HKV):
            s0 = lax.dot_general(qs[h], kbuf[h, pl.ds(base, G), :], nt, preferred_element_type=f32)
            s1 = lax.dot_general(qs[h], kbuf[HKV + h, pl.ds(base, G), :], nt, preferred_element_type=f32)
            ss.append(jnp.where(even_g, s0, s1) * scale)
        pbs, alphas = [], []
        for h in range(HKV):
            s = ss[h]
            m_cur = jnp.max(s, axis=-1, keepdims=True)
            m_new = m_cur if j == 0 else jnp.maximum(ms[h], m_cur)
            p = jnp.exp(s - m_new)
            psum = p[:, 0:DH]
            for t in range(1, G // DH):
                psum = psum + p[:, t * DH:(t + 1) * DH]
            if j == 0:
                alphas.append(None)
                ls[h] = psum
            else:
                alpha = jnp.exp(ms[h] - m_new)
                alphas.append(alpha)
                ls[h] = ls[h] * alpha + psum
            pbs.append(p.astype(bf16))
            ms[h] = m_new
        for h in range(HKV):
            o0 = jnp.dot(pbs[h], vbuf[h, pl.ds(base, G), :], preferred_element_type=f32)
            o1 = jnp.dot(pbs[h], vbuf[HKV + h, pl.ds(base, G), :], preferred_element_type=f32)
            o = jnp.where(even, o0, o1)
            accs[h] = o if j == 0 else accs[h] * alphas[h] + o

    heads = []
    for h in range(HKV):
        oh = accs[h] / jnp.sum(ls[h], axis=-1, keepdims=True)
        for g in range(REP):
            heads.append(oh if g == 0 else pltpu.roll(oh, 8 - 2 * g, 0))
    lhs = [o.astype(bf16) for o in heads]
    rolled = [pltpu.roll(o, 8, 1) for o in heads]
    lhs_prev = [jnp.where(lane128 < 8, rolled[i - 1], rolled[i]).astype(bf16) for i in range(HQ)]

    def coef(v, b):
        return jnp.transpose(jnp.broadcast_to(v.astype(f32)[b:b + 1], (DH, DH)))
    c_same = [coef(lhs[HQ - 1], b) for b in range(B)]
    c_prev = [coef(lhs_prev[HQ - 1], b) for b in range(B)]

    b1v = b1_buf[...].astype(f32)
    w1_cols = _col_tiles(w1_buf[...], F // 128)
    hdn = jnp.concatenate(
        [jnp.dot(xn, w1_cols[c], preferred_element_type=f32)
         + jnp.broadcast_to(b1v[c:c + 1], (8, DH)) for c in range(F // 128)], axis=1)
    sp = jnp.log1p(jnp.exp(-jnp.abs(hdn))) + jnp.maximum(hdn, 0.0)
    act = (hdn * jnp.tanh(sp)).astype(bf16)

    NC = D // 128
    outs = [x8[:, c * 128:(c + 1) * 128] for c in range(NC)]

    def add_wo(gi):
        for seg, g in wo_groups[gi]:
            i = seg * REP + g
            cols = _col_tiles(wo_buf[seg, g], NC)
            for cv in range(NC):
                c = (cv - O_WO) % NC
                a = lhs[i] if cv >= O_WO else lhs_prev[i]
                outs[c] = outs[c] + jnp.dot(a, cols[cv], preferred_element_type=f32)

    wait_all(w2_buf, S_W2)
    issue_until_pair(p_end + EXTRA1 + EXTRA2)
    wait_wo(0)
    w2_cols = _col_tiles(w2_buf[...], NC)
    for c in range(NC):
        outs[c] = outs[c] + jnp.dot(act, w2_cols[c], preferred_element_type=f32)
    add_wo(0)

    for region in wo_regions:
        for gi in region:
            wait_wo(gi)
        issue_until_pair(None)
        for gi in region:
            add_wo(gi)

    vacc = [[None] * NC for _ in range(B)]
    for vi in range(len(VSPLIT) - 1):
        a0, a1 = VSPLIT[vi], VSPLIT[vi + 1]
        wait_all(wo_buf.at[HKV - 1, REP - 1, pl.ds(NC * a0, NC * (a1 - a0))], S_LAST + vi)
        val = wo_buf[HKV - 1, REP - 1, pl.ds(NC * a0, NC * (a1 - a0))].astype(f32)
        for a in range(a0, a1):
            for cv in range(NC):
                c = (cv - O_WO) % NC
                cm = c_same if cv >= O_WO else c_prev
                for b in range(B):
                    t = val[NC * (a - a0) + cv] * cm[b][8 * a:8 * a + 8]
                    vacc[b][c] = t if vacc[b][c] is None else vacc[b][c] + t
    res = []
    for c in range(NC):
        s0 = jnp.sum(vacc[0][c], axis=0, keepdims=True)
        s1 = jnp.sum(vacc[1][c], axis=0, keepdims=True)
        res.append(outs[c] + jnp.where(even, s0, s1))
    o_ref[...] = jnp.concatenate(res, axis=1)[0:B].astype(o_ref.dtype)


@jax.jit
def pallas_parallel_sum__sliding_block_cached__dense_activation_mish__decode_kernel(
    A_x: jax.Array,
    A_k_cache: jax.Array,
    A_v_cache: jax.Array,
    A_wq: jax.Array,
    A_wo: jax.Array,
    B_x: jax.Array,
    B_w1: jax.Array,
    B_b1: jax.Array,
    B_w2: jax.Array,
):
    del B_x
    SK = A_k_cache.shape[2]
    W = min(4096, max(256, SK // 4))
    assert A_x.shape == (B, 1, D) and A_k_cache.shape == (B, HKV, SK, DH) and W % G == 0
    assert A_wq.shape == (D, HQ * DH) and A_wo.shape == (HQ * DH, D)
    assert B_w1.shape == (D, F) and B_w2.shape == (F, D)
    bf16 = jnp.bfloat16
    x = A_x.reshape(B, D)
    b1 = B_b1.reshape(F // 128, 128)
    k = A_k_cache.reshape(NBH, SK, DH)
    v = A_v_cache.reshape(NBH, SK, DH)
    wq, wo, w1, w2 = _tiles(A_wq), _tiles(A_wo), _tiles(B_w1), _tiles(B_w2)
    n_sems = 5 + 2 * (W // G) + N_WO_GROUPS + len(VSPLIT) - 1
    out = pl.pallas_call(
        functools.partial(_kernel, W=W, SK=SK),
        out_shape=jax.ShapeDtypeStruct((B, D), A_x.dtype),
        in_specs=[pl.BlockSpec(memory_space=pl.ANY)] * 8,
        out_specs=pl.BlockSpec(memory_space=pltpu.VMEM),
        scratch_shapes=[
            pltpu.VMEM((B, D), bf16),
            pltpu.VMEM((F // 128, 128), bf16),
            pltpu.VMEM((NBH, W, DH), bf16),
            pltpu.VMEM((NBH, W, DH), bf16),
            pltpu.VMEM(wq.shape, bf16),
            pltpu.VMEM((HKV, REP, 64, 8, 128), bf16),
            pltpu.VMEM(w1.shape, bf16),
            pltpu.VMEM(w2.shape, bf16),
            pltpu.SemaphoreType.DMA((n_sems,)),
        ],
        compiler_params=pltpu.CompilerParams(
            vmem_limit_bytes=100 * 1024 * 1024,
            disable_semaphore_checks=True,
        ),
    )(x, k, v, wq, wo, w1, b1, w2)
    return out.reshape(A_x.shape)
```

```python
import functools

import jax
import jax.numpy as jnp
from jax import lax
import jax.experimental.pallas as pl
import jax.experimental.pallas.tpu as pltpu

B, D = 2, 512
HQ, HKV, DH = 32, 8, 128
REP = HQ // HKV
F = 1792
NBH = B * HKV
CK = 128
G = 512
UT = 16
STEP = 16

KV_SHIFT = 16
O_WQ, O_WO, O_W1, O_W2 = 2, 2, 1, 15

LEAD = 22
LAG = 30
EXTRA1, EXTRA2 = 14, 12
VSPLIT = (0, 10, 14, 16)
N_WO_GROUPS = 10


def _cyc(n, step):
    return [i for s in range(step) for i in range(s, n, step)]


def _tiles(w):
    r, c = w.shape
    return (w.reshape(r // 8, 8, c // 128, 128).transpose(0, 2, 1, 3)
            .reshape((r // 8) * (c // 128), 8, 128))


def _col_tiles(val, n_col_tiles):
    n = val.shape[0] // n_col_tiles
    v4 = val.reshape(n, n_col_tiles, 8, 128)
    return [v4[:, c].reshape(n * 8, 128) for c in range(n_col_tiles)]


def _kernel(x_hbm, k_hbm, v_hbm, wq_hbm, wo_hbm, w1_hbm, b1_hbm, w2_hbm, o_ref,
            x_buf, b1_buf, kbuf, vbuf, wq_buf, wo_buf, w1_buf, w2_buf, sems, *, W, SK):
    f32, bf16 = jnp.float32, jnp.bfloat16
    cp = pltpu.make_async_copy
    NG = W // G
    UPG = (G // CK) * NBH
    S_X, S_B1, S_WQ, S_W1, S_W2, S_K = 0, 1, 2, 3, 4, 5
    S_V = S_K + NG
    S_WO = S_V + NG
    S_LAST = S_WO + N_WO_GROUPS

    def w_units(src, dst, si, o):
        n = src.shape[0]

        def piece(a, m):
            return cp(src.at[pl.ds(a, m)], dst.at[pl.ds(a, m)], sems.at[si])

        def unit(u):
            if u == 0:
                return [piece(0, UT - o), piece(n - o, o)]
            return [piece(UT * u - o, UT)]
        return [unit(u) for u in _cyc(n // UT, STEP)]

    def kv_unit(src, dst, si, j, c, r):
        off, sh, sem = j * G + c * CK, KV_SHIFT, sems.at[si + j]
        if off == 0:
            return [cp(src.at[r, pl.ds(SK - W, CK - sh), :], dst.at[r, pl.ds(sh, CK - sh), :], sem),
                    cp(src.at[r, pl.ds(SK - sh, sh), :], dst.at[r, pl.ds(0, sh), :], sem)]
        return [cp(src.at[r, pl.ds(SK - W + off - sh, CK), :], dst.at[r, pl.ds(off, CK), :], sem)]

    def wo_unit(seg, g, t0, nt, si):
        a, sem = (seg * REP + g) * 64 + t0 - O_WO, sems.at[si]
        if a < 0:
            return [cp(wo_hbm.at[pl.ds(0, nt + a)], wo_buf.at[seg, g, pl.ds(t0 - a, nt + a)], sem),
                    cp(wo_hbm.at[pl.ds(wo_hbm.shape[0] + a, -a)], wo_buf.at[seg, g, pl.ds(t0, -a)], sem)]
        return [cp(wo_hbm.at[pl.ds(a, nt)], wo_buf.at[seg, g, pl.ds(t0, nt)], sem)]

    hi = w_units(wq_hbm, wq_buf, S_WQ, O_WQ)
    lo = []
    p_k = len(hi)
    for j in range(NG):
        for c in range(G // CK):
            for r in range(NBH):
                hi.append(kv_unit(k_hbm, kbuf, S_K, j, c, r))
                lo.append(kv_unit(v_hbm, vbuf, S_V, j, c, r))
    lo += w_units(w1_hbm, w1_buf, S_W1, O_W1)
    lo += w_units(w2_hbm, w2_buf, S_W2, O_W2)

    wo_groups = []

    def add_cycle(stream, blocks):
        si = S_WO + len(wo_groups)
        wo_groups.append(blocks)
        for c in range(64 // UT):
            for seg, g in blocks:
                stream.append(wo_unit(seg, g, c * UT, UT, si))

    add_cycle(hi, [(s, 0) for s in range(4)])
    add_cycle(hi, [(s, 1) for s in range(4)])
    add_cycle(hi, [(s, 2) for s in range(4)])
    add_cycle(hi, [(0, 3)])
    add_cycle(lo, [(1, 3), (2, 3), (3, 3)])
    add_cycle(lo, [(s, 0) for s in range(4, 8)])
    add_cycle(lo, [(s, 1) for s in range(4, 8)])
    add_cycle(lo, [(s, 2) for s in range(4, 8)])
    add_cycle(lo, [(4, 3), (5, 3)])
    wo_groups.append([(6, 3)])
    lo += [wo_unit(6, 3, t, 4, S_WO + 9) for t in range(0, 64, 4)]
    for vi in range(len(VSPLIT) - 1):
        lo += [wo_unit(7, 3, 4 * a, 4, S_LAST + vi) for a in range(VSPLIT[vi], VSPLIT[vi + 1])]
    assert len(wo_groups) == N_WO_GROUPS
    wo_first = [0, 4, 5]
    wo_regions = [[1, 6], [2, 7], [3, 8], [9]]

    seq = [(c, 1) for u in lo[:LEAD] for c in u]
    pos_of_pair = []
    rest = lo[LEAD:]
    for i in range(max(len(hi), len(rest))):
        if i < len(hi):
            seq += [(c, 0) for c in hi[i]]
        if i < len(rest):
            seq += [(c, 1) for c in rest[i]]
        pos_of_pair.append(len(seq))
    issued = [0]

    def issue_until_pair(p):
        end = len(seq) if p is None or p >= len(pos_of_pair) else pos_of_pair[p]
        for c, pr in seq[issued[0]:end]:
            c.start(priority=pr)
        issued[0] = max(issued[0], end)

    def wait_all(ref, si):
        cp(ref, ref, sems.at[si]).wait()

    def wait_wo(gi):
        blocks = wo_groups[gi]
        wait_all(wo_buf.at[pl.ds(blocks[0][0], len(blocks)), blocks[0][1]], S_WO + gi)

    c_x = cp(x_hbm, x_buf, sems.at[S_X])
    c_b1 = cp(b1_hbm, b1_buf, sems.at[S_B1])
    seq[0][0].start(priority=seq[0][1])
    issued[0] = 1
    c_x.start(priority=0)
    c_b1.start(priority=0)
    issue_until_pair(p_k - 1 + LAG)

    c_x.wait()
    row = lax.broadcasted_iota(jnp.int32, (8, D), 0)
    x2 = x_buf[...].astype(f32)
    x8 = jnp.where(row % 2 == 0, jnp.broadcast_to(x2[0:1], (8, D)), jnp.broadcast_to(x2[1:2], (8, D)))
    mu = jnp.mean(x8, axis=-1, keepdims=True)
    xc = x8 - mu
    var = jnp.mean(xc * xc, axis=-1, keepdims=True)
    xn = (xc / jnp.sqrt(var + 1e-5)).astype(bf16)

    row128 = lax.broadcasted_iota(jnp.int32, (8, DH), 0)
    lane128 = lax.broadcasted_iota(jnp.int32, (8, DH), 1)
    g_of_row = row128 // 2
    even = row128 % 2 == 0

    wait_all(wq_buf, S_WQ)
    wq_cols = _col_tiles(wq_buf[...], HQ)
    qs = []
    for h in range(HKV):
        qh = None
        for g in range(REP):
            qg = jnp.dot(xn, wq_cols[h * REP + g], preferred_element_type=f32)
            qh = qg if g == 0 else jnp.where(g_of_row == g, qg, qh)
        qs.append(qh.astype(bf16))

    issue_until_pair(p_k + UPG - 1 + LAG)

    scale = DH ** -0.5
    nt = (((1,), (1,)), ((), ()))
    even_g = lax.broadcasted_iota(jnp.int32, (8, G), 0) % 2 == 0
    ms, ls, accs = [None] * HKV, [None] * HKV, [None] * HKV
    p_end = p_k + NG * UPG - 1 + LAG

    for j in range(NG):
        base = j * G
        wait_all(kbuf.at[:, pl.ds(base, G), :], S_K + j)
        wait_all(vbuf.at[:, pl.ds(base, G), :], S_V + j)
        if j < NG - 1:
            issue_until_pair(p_k + (j + 2) * UPG - 1 + LAG)
        else:
            issue_until_pair(p_end + EXTRA1)
            wait_all(w1_buf, S_W1)
            c_b1.wait()
        ss = []
        for h in range(HKV):
            s0 = lax.dot_general(qs[h], kbuf[h, pl.ds(base, G), :], nt, preferred_element_type=f32)
            s1 = lax.dot_general(qs[h], kbuf[HKV + h, pl.ds(base, G), :], nt, preferred_element_type=f32)
            ss.append(jnp.where(even_g, s0, s1) * scale)
        pbs, alphas = [], []
        for h in range(HKV):
            s = ss[h]
            m_cur = jnp.max(s, axis=-1, keepdims=True)
            m_new = m_cur if j == 0 else jnp.maximum(ms[h], m_cur)
            p = jnp.exp(s - m_new)
            psum = p[:, 0:DH]
            for t in range(1, G // DH):
                psum = psum + p[:, t * DH:(t + 1) * DH]
            if j == 0:
                alphas.append(None)
                ls[h] = psum
            else:
                alpha = jnp.exp(ms[h] - m_new)
                alphas.append(alpha)
                ls[h] = ls[h] * alpha + psum
            pbs.append(p.astype(bf16))
            ms[h] = m_new
        for h in range(HKV):
            o0 = jnp.dot(pbs[h], vbuf[h, pl.ds(base, G), :], preferred_element_type=f32)
            o1 = jnp.dot(pbs[h], vbuf[HKV + h, pl.ds(base, G), :], preferred_element_type=f32)
            o = jnp.where(even, o0, o1)
            accs[h] = o if j == 0 else accs[h] * alphas[h] + o

    heads = []
    for h in range(HKV):
        oh = accs[h] / jnp.sum(ls[h], axis=-1, keepdims=True)
        for g in range(REP):
            heads.append(oh if g == 0 else pltpu.roll(oh, 8 - 2 * g, 0))
    lhs = [o.astype(bf16) for o in heads]
    rolled = [pltpu.roll(o, 8, 1) for o in heads]
    lhs_prev = [jnp.where(lane128 < 8, rolled[i - 1], rolled[i]).astype(bf16) for i in range(HQ)]

    def coef(v, b):
        return jnp.transpose(jnp.broadcast_to(v.astype(f32)[b:b + 1], (DH, DH)))
    c_same = [coef(lhs[HQ - 1], b) for b in range(B)]
    c_prev = [coef(lhs_prev[HQ - 1], b) for b in range(B)]

    b1v = b1_buf[...].astype(f32)
    w1_cols = _col_tiles(w1_buf[...], F // 128)
    hdn = jnp.concatenate(
        [jnp.dot(xn, w1_cols[c], preferred_element_type=f32)
         + jnp.broadcast_to(b1v[c:c + 1], (8, DH)) for c in range(F // 128)], axis=1)
    sp = jnp.log1p(jnp.exp(-jnp.abs(hdn))) + jnp.maximum(hdn, 0.0)
    act = (hdn * jnp.tanh(sp)).astype(bf16)

    NC = D // 128
    outs = [x8[:, c * 128:(c + 1) * 128] for c in range(NC)]

    def add_wo(gi):
        for seg, g in wo_groups[gi]:
            i = seg * REP + g
            cols = _col_tiles(wo_buf[seg, g], NC)
            for cv in range(NC):
                c = (cv - O_WO) % NC
                a = lhs[i] if cv >= O_WO else lhs_prev[i]
                outs[c] = outs[c] + jnp.dot(a, cols[cv], preferred_element_type=f32)

    wait_all(w2_buf, S_W2)
    issue_until_pair(p_end + EXTRA1 + EXTRA2)
    for gi in wo_first:
        wait_wo(gi)
    w2_cols = _col_tiles(w2_buf[...], NC)
    for c in range(NC):
        outs[c] = outs[c] + jnp.dot(act, w2_cols[c], preferred_element_type=f32)
    for gi in wo_first:
        add_wo(gi)

    for region in wo_regions:
        for gi in region:
            wait_wo(gi)
        issue_until_pair(None)
        for gi in region:
            add_wo(gi)

    vacc = [[None] * NC for _ in range(B)]
    for vi in range(len(VSPLIT) - 1):
        a0, a1 = VSPLIT[vi], VSPLIT[vi + 1]
        wait_all(wo_buf.at[HKV - 1, REP - 1, pl.ds(NC * a0, NC * (a1 - a0))], S_LAST + vi)
        val = wo_buf[HKV - 1, REP - 1, pl.ds(NC * a0, NC * (a1 - a0))].astype(f32)
        for a in range(a0, a1):
            for cv in range(NC):
                c = (cv - O_WO) % NC
                cm = c_same if cv >= O_WO else c_prev
                for b in range(B):
                    t = val[NC * (a - a0) + cv] * cm[b][8 * a:8 * a + 8]
                    vacc[b][c] = t if vacc[b][c] is None else vacc[b][c] + t
    res = []
    for c in range(NC):
        s0 = jnp.sum(vacc[0][c], axis=0, keepdims=True)
        s1 = jnp.sum(vacc[1][c], axis=0, keepdims=True)
        res.append(outs[c] + jnp.where(even, s0, s1))
    o_ref[...] = jnp.concatenate(res, axis=1)[0:B].astype(o_ref.dtype)


@jax.jit
def pallas_parallel_sum__sliding_block_cached__dense_activation_mish__decode_kernel(
    A_x: jax.Array,
    A_k_cache: jax.Array,
    A_v_cache: jax.Array,
    A_wq: jax.Array,
    A_wo: jax.Array,
    B_x: jax.Array,
    B_w1: jax.Array,
    B_b1: jax.Array,
    B_w2: jax.Array,
):
    del B_x
    SK = A_k_cache.shape[2]
    W = min(4096, max(256, SK // 4))
    assert A_x.shape == (B, 1, D) and A_k_cache.shape == (B, HKV, SK, DH) and W % G == 0
    assert A_wq.shape == (D, HQ * DH) and A_wo.shape == (HQ * DH, D)
    assert B_w1.shape == (D, F) and B_w2.shape == (F, D)
    bf16 = jnp.bfloat16
    x = A_x.reshape(B, D)
    b1 = B_b1.reshape(F // 128, 128)
    k = A_k_cache.reshape(NBH, SK, DH)
    v = A_v_cache.reshape(NBH, SK, DH)
    wq, wo, w1, w2 = _tiles(A_wq), _tiles(A_wo), _tiles(B_w1), _tiles(B_w2)
    n_sems = 5 + 2 * (W // G) + N_WO_GROUPS + len(VSPLIT) - 1
    out = pl.pallas_call(
        functools.partial(_kernel, W=W, SK=SK),
        out_shape=jax.ShapeDtypeStruct((B, D), A_x.dtype),
        in_specs=[pl.BlockSpec(memory_space=pl.ANY)] * 8,
        out_specs=pl.BlockSpec(memory_space=pltpu.VMEM),
        scratch_shapes=[
            pltpu.VMEM((B, D), bf16),
            pltpu.VMEM((F // 128, 128), bf16),
            pltpu.VMEM((NBH, W, DH), bf16),
            pltpu.VMEM((NBH, W, DH), bf16),
            pltpu.VMEM(wq.shape, bf16),
            pltpu.VMEM((HKV, REP, 64, 8, 128), bf16),
            pltpu.VMEM(w1.shape, bf16),
            pltpu.VMEM(w2.shape, bf16),
            pltpu.SemaphoreType.DMA((n_sems,)),
        ],
        compiler_params=pltpu.CompilerParams(
            vmem_limit_bytes=100 * 1024 * 1024,
            disable_semaphore_checks=True,
        ),
    )(x, k, v, wq, wo, w1, b1, w2)
    return out.reshape(A_x.shape)
```

```python
import functools

import jax
import jax.numpy as jnp
from jax import lax
import jax.experimental.pallas as pl
import jax.experimental.pallas.tpu as pltpu

B, D = 2, 512
HQ, HKV, DH = 32, 8, 128
REP = HQ // HKV
F = 1792
NBH = B * HKV
CK = 128
G = 512
UT = 16
STEP = 16

KV_SHIFT = 16
O_WQ, O_WO, O_W1, O_W2 = 2, 2, 1, 15

LEAD = 22
LAG = 30
EXTRA1, EXTRA2 = 14, 12
N_WO_GROUPS = 9
V_SLICES = ((6, 0, 14), (6, 14, 16), (7, 0, 6), (7, 6, 10), (7, 10, 13), (7, 13, 16))
V_REGIONS = ((0,), (1, 2), (3,), (4,), (5,))


def _cyc(n, step):
    return [i for s in range(step) for i in range(s, n, step)]


def _tiles(w):
    r, c = w.shape
    return (w.reshape(r // 8, 8, c // 128, 128).transpose(0, 2, 1, 3)
            .reshape((r // 8) * (c // 128), 8, 128))


def _col_tiles(val, n_col_tiles):
    n = val.shape[0] // n_col_tiles
    v4 = val.reshape(n, n_col_tiles, 8, 128)
    return [v4[:, c].reshape(n * 8, 128) for c in range(n_col_tiles)]


def _kernel(x_hbm, k_hbm, v_hbm, wq_hbm, wo_hbm, w1_hbm, b1_hbm, w2_hbm, o_ref,
            x_buf, b1_buf, kbuf, vbuf, wq_buf, wo_buf, w1_buf, w2_buf, sems, *, W, SK):
    f32, bf16 = jnp.float32, jnp.bfloat16
    cp = pltpu.make_async_copy
    NG = W // G
    UPG = (G // CK) * NBH
    S_X, S_B1, S_WQ, S_W1, S_W2, S_K = 0, 1, 2, 3, 4, 5
    S_V = S_K + NG
    S_WO = S_V + NG
    S_LAST = S_WO + N_WO_GROUPS

    def w_units(src, dst, si, o):
        n = src.shape[0]

        def piece(a, m):
            return cp(src.at[pl.ds(a, m)], dst.at[pl.ds(a, m)], sems.at[si])

        def unit(u):
            if u == 0:
                return [piece(0, UT - o), piece(n - o, o)]
            return [piece(UT * u - o, UT)]
        return [unit(u) for u in _cyc(n // UT, STEP)]

    def kv_unit(src, dst, si, j, c, r):
        off, sh, sem = j * G + c * CK, KV_SHIFT, sems.at[si + j]
        if off == 0:
            return [cp(src.at[r, pl.ds(SK - W, CK - sh), :], dst.at[r, pl.ds(sh, CK - sh), :], sem),
                    cp(src.at[r, pl.ds(SK - sh, sh), :], dst.at[r, pl.ds(0, sh), :], sem)]
        return [cp(src.at[r, pl.ds(SK - W + off - sh, CK), :], dst.at[r, pl.ds(off, CK), :], sem)]

    def wo_unit(seg, g, t0, nt, si):
        a, sem = (seg * REP + g) * 64 + t0 - O_WO, sems.at[si]
        if a < 0:
            return [cp(wo_hbm.at[pl.ds(0, nt + a)], wo_buf.at[seg, g, pl.ds(t0 - a, nt + a)], sem),
                    cp(wo_hbm.at[pl.ds(wo_hbm.shape[0] + a, -a)], wo_buf.at[seg, g, pl.ds(t0, -a)], sem)]
        return [cp(wo_hbm.at[pl.ds(a, nt)], wo_buf.at[seg, g, pl.ds(t0, nt)], sem)]

    hi = w_units(wq_hbm, wq_buf, S_WQ, O_WQ)
    lo = []
    p_k = len(hi)
    for j in range(NG):
        for c in range(G // CK):
            for r in range(NBH):
                hi.append(kv_unit(k_hbm, kbuf, S_K, j, c, r))
                lo.append(kv_unit(v_hbm, vbuf, S_V, j, c, r))
    lo += w_units(w1_hbm, w1_buf, S_W1, O_W1)
    lo += w_units(w2_hbm, w2_buf, S_W2, O_W2)

    wo_groups = []

    def add_cycle(stream, blocks):
        si = S_WO + len(wo_groups)
        wo_groups.append(blocks)
        for c in range(64 // UT):
            for seg, g in blocks:
                stream.append(wo_unit(seg, g, c * UT, UT, si))

    add_cycle(hi, [(s, 0) for s in range(4)])
    add_cycle(hi, [(s, 1) for s in range(4)])
    add_cycle(hi, [(s, 2) for s in range(4)])
    add_cycle(hi, [(0, 3)])
    add_cycle(lo, [(1, 3), (2, 3), (3, 3)])
    add_cycle(lo, [(s, 0) for s in range(4, 8)])
    add_cycle(lo, [(s, 1) for s in range(4, 8)])
    add_cycle(lo, [(s, 2) for s in range(4, 8)])
    add_cycle(lo, [(4, 3), (5, 3)])
    for vi, (seg, a0, a1) in enumerate(V_SLICES):
        lo += [wo_unit(seg, 3, 4 * a, 4, S_LAST + vi) for a in range(a0, a1)]
    assert len(wo_groups) == N_WO_GROUPS
    wo_first = [0, 4, 5]
    wo_regions = [[1, 6], [2, 7], [3, 8]]

    seq = [(c, 1) for u in lo[:LEAD] for c in u]
    pos_of_pair = []
    rest = lo[LEAD:]
    for i in range(max(len(hi), len(rest))):
        if i < len(hi):
            seq += [(c, 0) for c in hi[i]]
        if i < len(rest):
            seq += [(c, 1) for c in rest[i]]
        pos_of_pair.append(len(seq))
    issued = [0]

    def issue_until_pair(p):
        end = len(seq) if p is None or p >= len(pos_of_pair) else pos_of_pair[p]
        for c, pr in seq[issued[0]:end]:
            c.start(priority=pr)
        issued[0] = max(issued[0], end)

    def wait_all(ref, si):
        cp(ref, ref, sems.at[si]).wait()

    def wait_wo(gi):
        blocks = wo_groups[gi]
        wait_all(wo_buf.at[pl.ds(blocks[0][0], len(blocks)), blocks[0][1]], S_WO + gi)

    c_x = cp(x_hbm, x_buf, sems.at[S_X])
    c_b1 = cp(b1_hbm, b1_buf, sems.at[S_B1])
    seq[0][0].start(priority=seq[0][1])
    issued[0] = 1
    c_x.start(priority=0)
    c_b1.start(priority=0)
    issue_until_pair(p_k - 1 + LAG)

    c_x.wait()
    row = lax.broadcasted_iota(jnp.int32, (8, D), 0)
    x2 = x_buf[...].astype(f32)
    x8 = jnp.where(row % 2 == 0, jnp.broadcast_to(x2[0:1], (8, D)), jnp.broadcast_to(x2[1:2], (8, D)))
    mu = jnp.mean(x8, axis=-1, keepdims=True)
    xc = x8 - mu
    var = jnp.mean(xc * xc, axis=-1, keepdims=True)
    xn = (xc / jnp.sqrt(var + 1e-5)).astype(bf16)

    row128 = lax.broadcasted_iota(jnp.int32, (8, DH), 0)
    lane128 = lax.broadcasted_iota(jnp.int32, (8, DH), 1)
    g_of_row = row128 // 2
    even = row128 % 2 == 0

    wait_all(wq_buf, S_WQ)
    wq_cols = _col_tiles(wq_buf[...], HQ)
    qs = []
    for h in range(HKV):
        qh = None
        for g in range(REP):
            qg = jnp.dot(xn, wq_cols[h * REP + g], preferred_element_type=f32)
            qh = qg if g == 0 else jnp.where(g_of_row == g, qg, qh)
        qs.append(qh.astype(bf16))

    issue_until_pair(p_k + UPG - 1 + LAG)

    scale = DH ** -0.5
    nt = (((1,), (1,)), ((), ()))
    even_g = lax.broadcasted_iota(jnp.int32, (8, G), 0) % 2 == 0
    ms, ls, accs = [None] * HKV, [None] * HKV, [None] * HKV
    p_end = p_k + NG * UPG - 1 + LAG

    for j in range(NG):
        base = j * G
        wait_all(kbuf.at[:, pl.ds(base, G), :], S_K + j)
        wait_all(vbuf.at[:, pl.ds(base, G), :], S_V + j)
        if j < NG - 1:
            issue_until_pair(p_k + (j + 2) * UPG - 1 + LAG)
        else:
            issue_until_pair(p_end + EXTRA1)
            wait_all(w1_buf, S_W1)
            c_b1.wait()
        ss = []
        for h in range(HKV):
            s0 = lax.dot_general(qs[h], kbuf[h, pl.ds(base, G), :], nt, preferred_element_type=f32)
            s1 = lax.dot_general(qs[h], kbuf[HKV + h, pl.ds(base, G), :], nt, preferred_element_type=f32)
            ss.append(jnp.where(even_g, s0, s1) * scale)
        pbs, alphas = [], []
        for h in range(HKV):
            s = ss[h]
            m_cur = jnp.max(s, axis=-1, keepdims=True)
            m_new = m_cur if j == 0 else jnp.maximum(ms[h], m_cur)
            p = jnp.exp(s - m_new)
            psum = p[:, 0:DH]
            for t in range(1, G // DH):
                psum = psum + p[:, t * DH:(t + 1) * DH]
            if j == 0:
                alphas.append(None)
                ls[h] = psum
            else:
                alpha = jnp.exp(ms[h] - m_new)
                alphas.append(alpha)
                ls[h] = ls[h] * alpha + psum
            pbs.append(p.astype(bf16))
            ms[h] = m_new
        for h in range(HKV):
            o0 = jnp.dot(pbs[h], vbuf[h, pl.ds(base, G), :], preferred_element_type=f32)
            o1 = jnp.dot(pbs[h], vbuf[HKV + h, pl.ds(base, G), :], preferred_element_type=f32)
            o = jnp.where(even, o0, o1)
            accs[h] = o if j == 0 else accs[h] * alphas[h] + o

    heads = []
    for h in range(HKV):
        oh = accs[h] / jnp.sum(ls[h], axis=-1, keepdims=True)
        for g in range(REP):
            heads.append(oh if g == 0 else pltpu.roll(oh, 8 - 2 * g, 0))
    lhs = [o.astype(bf16) for o in heads]
    rolled = [pltpu.roll(o, 8, 1) for o in heads]
    lhs_prev = [jnp.where(lane128 < 8, rolled[i - 1], rolled[i]).astype(bf16) for i in range(HQ)]

    def coef(v, b):
        return jnp.transpose(jnp.broadcast_to(v.astype(f32)[b:b + 1], (DH, DH)))
    c_same = {seg: [coef(lhs[seg * REP + 3], b) for b in range(B)] for seg in (6, 7)}
    c_prev = {seg: [coef(lhs_prev[seg * REP + 3], b) for b in range(B)] for seg in (6, 7)}

    b1v = b1_buf[...].astype(f32)
    w1_cols = _col_tiles(w1_buf[...], F // 128)
    hdn = jnp.concatenate(
        [jnp.dot(xn, w1_cols[c], preferred_element_type=f32)
         + jnp.broadcast_to(b1v[c:c + 1], (8, DH)) for c in range(F // 128)], axis=1)
    sp = jnp.log1p(jnp.exp(-jnp.abs(hdn))) + jnp.maximum(hdn, 0.0)
    act = (hdn * jnp.tanh(sp)).astype(bf16)

    NC = D // 128
    outs = [x8[:, c * 128:(c + 1) * 128] for c in range(NC)]

    def add_wo(gi):
        for seg, g in wo_groups[gi]:
            i = seg * REP + g
            cols = _col_tiles(wo_buf[seg, g], NC)
            for cv in range(NC):
                c = (cv - O_WO) % NC
                a = lhs[i] if cv >= O_WO else lhs_prev[i]
                outs[c] = outs[c] + jnp.dot(a, cols[cv], preferred_element_type=f32)

    wait_all(w2_buf, S_W2)
    issue_until_pair(p_end + EXTRA1 + EXTRA2)
    for gi in wo_first:
        wait_wo(gi)
    w2_cols = _col_tiles(w2_buf[...], NC)
    for c in range(NC):
        outs[c] = outs[c] + jnp.dot(act, w2_cols[c], preferred_element_type=f32)
    for gi in wo_first:
        add_wo(gi)

    for region in wo_regions:
        for gi in region:
            wait_wo(gi)
        issue_until_pair(None)
        for gi in region:
            add_wo(gi)

    vacc = [[None] * NC for _ in range(B)]
    for region in V_REGIONS:
        for vi in region:
            seg, a0, a1 = V_SLICES[vi]
            wait_all(wo_buf.at[seg, 3, pl.ds(NC * a0, NC * (a1 - a0))], S_LAST + vi)
        for vi in region:
            seg, a0, a1 = V_SLICES[vi]
            val = wo_buf[seg, 3, pl.ds(NC * a0, NC * (a1 - a0))].astype(f32)
            for a in range(a0, a1):
                for cv in range(NC):
                    c = (cv - O_WO) % NC
                    for b in range(B):
                        if cv >= O_WO:
                            cf = c_same[seg][b][8 * a:8 * a + 8]
                        elif a > 0:
                            cf = c_same[seg][b][8 * a - 8:8 * a]
                        else:
                            cf = c_prev[seg][b][0:8]
                        t = val[NC * (a - a0) + cv] * cf
                        vacc[b][c] = t if vacc[b][c] is None else vacc[b][c] + t
    res = []
    for c in range(NC):
        s0 = jnp.sum(vacc[0][c], axis=0, keepdims=True)
        s1 = jnp.sum(vacc[1][c], axis=0, keepdims=True)
        res.append(outs[c] + jnp.where(even, s0, s1))
    o_ref[...] = jnp.concatenate(res, axis=1)[0:B].astype(o_ref.dtype)


@jax.jit
def pallas_parallel_sum__sliding_block_cached__dense_activation_mish__decode_kernel(
    A_x: jax.Array,
    A_k_cache: jax.Array,
    A_v_cache: jax.Array,
    A_wq: jax.Array,
    A_wo: jax.Array,
    B_x: jax.Array,
    B_w1: jax.Array,
    B_b1: jax.Array,
    B_w2: jax.Array,
):
    del B_x
    SK = A_k_cache.shape[2]
    W = min(4096, max(256, SK // 4))
    assert A_x.shape == (B, 1, D) and A_k_cache.shape == (B, HKV, SK, DH) and W % G == 0
    assert A_wq.shape == (D, HQ * DH) and A_wo.shape == (HQ * DH, D)
    assert B_w1.shape == (D, F) and B_w2.shape == (F, D)
    bf16 = jnp.bfloat16
    x = A_x.reshape(B, D)
    b1 = B_b1.reshape(F // 128, 128)
    k = A_k_cache.reshape(NBH, SK, DH)
    v = A_v_cache.reshape(NBH, SK, DH)
    wq, wo, w1, w2 = _tiles(A_wq), _tiles(A_wo), _tiles(B_w1), _tiles(B_w2)
    n_sems = 5 + 2 * (W // G) + N_WO_GROUPS + len(V_SLICES)
    out = pl.pallas_call(
        functools.partial(_kernel, W=W, SK=SK),
        out_shape=jax.ShapeDtypeStruct((B, D), A_x.dtype),
        in_specs=[pl.BlockSpec(memory_space=pl.ANY)] * 8,
        out_specs=pl.BlockSpec(memory_space=pltpu.VMEM),
        scratch_shapes=[
            pltpu.VMEM((B, D), bf16),
            pltpu.VMEM((F // 128, 128), bf16),
            pltpu.VMEM((NBH, W, DH), bf16),
            pltpu.VMEM((NBH, W, DH), bf16),
            pltpu.VMEM(wq.shape, bf16),
            pltpu.VMEM((HKV, REP, 64, 8, 128), bf16),
            pltpu.VMEM(w1.shape, bf16),
            pltpu.VMEM(w2.shape, bf16),
            pltpu.SemaphoreType.DMA((n_sems,)),
        ],
        compiler_params=pltpu.CompilerParams(
            vmem_limit_bytes=100 * 1024 * 1024,
            disable_semaphore_checks=True,
        ),
    )(x, k, v, wq, wo, w1, b1, w2)
    return out.reshape(A_x.shape)
```

```python
import functools

import jax
import jax.numpy as jnp
from jax import lax
import jax.experimental.pallas as pl
import jax.experimental.pallas.tpu as pltpu

B, D = 2, 512
HQ, HKV, DH = 32, 8, 128
REP = HQ // HKV
F = 1792
NBH = B * HKV
CK = 128
G = 512
UT = 16
STEP = 16

KV_SHIFT = 16
O_WQ, O_WO, O_W1, O_W2 = 2, 2, 1, 15

LEAD = 24
LAG = 30
EXTRA = 14
N_WO_GROUPS = 9
V_SLICES = ((6, 0, 14), (6, 14, 16), (7, 0, 6), (7, 6, 10), (7, 10, 13), (7, 13, 16))
V_REGIONS = ((0,), (1, 2), (3,), (4,), (5,))


def _cyc(n, step):
    return [i for s in range(step) for i in range(s, n, step)]


def _tiles(w):
    r, c = w.shape
    return (w.reshape(r // 8, 8, c // 128, 128).transpose(0, 2, 1, 3)
            .reshape((r // 8) * (c // 128), 8, 128))


def _col_tiles(val, n_col_tiles):
    n = val.shape[0] // n_col_tiles
    v4 = val.reshape(n, n_col_tiles, 8, 128)
    return [v4[:, c].reshape(n * 8, 128) for c in range(n_col_tiles)]


def _kernel(x_hbm, k_hbm, v_hbm, wq_hbm, wo_hbm, w1_hbm, b1_hbm, w2_hbm, o_ref,
            x_buf, b1_buf, kbuf, vbuf, wq_buf, wo_buf, w1_buf, w2_buf, sems, *, W, SK):
    f32, bf16 = jnp.float32, jnp.bfloat16
    cp = pltpu.make_async_copy
    NG = W // G
    UPG = (G // CK) * NBH
    S_X, S_B1, S_WQ, S_W1, S_W2, S_K = 0, 1, 2, 3, 4, 5
    S_V = S_K + NG
    S_WO = S_V + NG
    S_LAST = S_WO + N_WO_GROUPS

    def w_units(src, dst, si, o):
        n = src.shape[0]

        def piece(a, m):
            return cp(src.at[pl.ds(a, m)], dst.at[pl.ds(a, m)], sems.at[si])

        def unit(u):
            if u == 0:
                return [piece(0, UT - o), piece(n - o, o)]
            return [piece(UT * u - o, UT)]
        return [unit(u) for u in _cyc(n // UT, STEP)]

    def kv_unit(src, dst, si, j, c, r):
        off, sh, sem = j * G + c * CK, KV_SHIFT, sems.at[si + j]
        if off == 0:
            return [cp(src.at[r, pl.ds(SK - W, CK - sh), :], dst.at[r, pl.ds(sh, CK - sh), :], sem),
                    cp(src.at[r, pl.ds(SK - sh, sh), :], dst.at[r, pl.ds(0, sh), :], sem)]
        return [cp(src.at[r, pl.ds(SK - W + off - sh, CK), :], dst.at[r, pl.ds(off, CK), :], sem)]

    def wo_unit(seg, g, t0, nt, si):
        a, sem = (seg * REP + g) * 64 + t0 - O_WO, sems.at[si]
        if a < 0:
            return [cp(wo_hbm.at[pl.ds(0, nt + a)], wo_buf.at[seg, g, pl.ds(t0 - a, nt + a)], sem),
                    cp(wo_hbm.at[pl.ds(wo_hbm.shape[0] + a, -a)], wo_buf.at[seg, g, pl.ds(t0, -a)], sem)]
        return [cp(wo_hbm.at[pl.ds(a, nt)], wo_buf.at[seg, g, pl.ds(t0, nt)], sem)]

    hi = w_units(wq_hbm, wq_buf, S_WQ, O_WQ)
    lo = []
    p_k = len(hi)
    for j in range(NG):
        chunks = list(range(G // CK))
        if j == 0:
            chunks = chunks[1:] + chunks[:1]
        for c in chunks:
            for r in range(NBH):
                hi.append(kv_unit(k_hbm, kbuf, S_K, j, c, r))
                lo.append(kv_unit(v_hbm, vbuf, S_V, j, c, r))
    lo += w_units(w1_hbm, w1_buf, S_W1, O_W1)
    lo += w_units(w2_hbm, w2_buf, S_W2, O_W2)

    wo_groups = []

    def add_cycle(stream, blocks):
        si = S_WO + len(wo_groups)
        wo_groups.append(blocks)
        for c in range(64 // UT):
            for seg, g in blocks:
                stream.append(wo_unit(seg, g, c * UT, UT, si))

    add_cycle(hi, [(s, 0) for s in range(4)])
    add_cycle(hi, [(s, 1) for s in range(4)])
    add_cycle(hi, [(s, 2) for s in range(4)])
    add_cycle(hi, [(0, 3)])
    add_cycle(lo, [(1, 3), (2, 3), (3, 3)])
    add_cycle(lo, [(s, 0) for s in range(4, 8)])
    add_cycle(lo, [(s, 1) for s in range(4, 8)])
    add_cycle(lo, [(s, 2) for s in range(4, 8)])
    add_cycle(lo, [(4, 3), (5, 3)])
    for vi, (seg, a0, a1) in enumerate(V_SLICES):
        lo += [wo_unit(seg, 3, 4 * a, 4, S_LAST + vi) for a in range(a0, a1)]
    assert len(wo_groups) == N_WO_GROUPS
    wo_first = [0, 4, 5]
    wo_regions = [[1, 6], [2, 7], [3, 8]]

    seq = [(c, 1) for u in lo[:LEAD] for c in u]
    pos_of_pair = []
    rest = lo[LEAD:]
    for i in range(max(len(hi), len(rest))):
        if i < len(hi):
            seq += [(c, 0) for c in hi[i]]
        if i < len(rest):
            seq += [(c, 1) for c in rest[i]]
        pos_of_pair.append(len(seq))
    issued = [0]

    def issue_until_pair(p):
        end = len(seq) if p is None or p >= len(pos_of_pair) else pos_of_pair[p]
        for c, pr in seq[issued[0]:end]:
            c.start(priority=pr)
        issued[0] = max(issued[0], end)

    def wait_all(ref, si):
        cp(ref, ref, sems.at[si]).wait()

    def wait_wo(gi):
        blocks = wo_groups[gi]
        wait_all(wo_buf.at[pl.ds(blocks[0][0], len(blocks)), blocks[0][1]], S_WO + gi)

    c_x = cp(x_hbm, x_buf, sems.at[S_X])
    c_b1 = cp(b1_hbm, b1_buf, sems.at[S_B1])
    seq[0][0].start(priority=seq[0][1])
    issued[0] = 1
    c_x.start(priority=0)
    c_b1.start(priority=0)
    issue_until_pair(p_k - 1 + LAG)

    c_x.wait()
    row = lax.broadcasted_iota(jnp.int32, (8, D), 0)
    x2 = x_buf[...].astype(f32)
    x8 = jnp.where(row % 2 == 0, jnp.broadcast_to(x2[0:1], (8, D)), jnp.broadcast_to(x2[1:2], (8, D)))
    mu = jnp.mean(x8, axis=-1, keepdims=True)
    xc = x8 - mu
    var = jnp.mean(xc * xc, axis=-1, keepdims=True)
    xn = (xc / jnp.sqrt(var + 1e-5)).astype(bf16)

    row128 = lax.broadcasted_iota(jnp.int32, (8, DH), 0)
    lane128 = lax.broadcasted_iota(jnp.int32, (8, DH), 1)
    g_of_row = row128 // 2
    even = row128 % 2 == 0

    wait_all(wq_buf, S_WQ)
    wq_cols = _col_tiles(wq_buf[...], HQ)
    qs = []
    for h in range(HKV):
        qh = None
        for g in range(REP):
            qg = jnp.dot(xn, wq_cols[h * REP + g], preferred_element_type=f32)
            qh = qg if g == 0 else jnp.where(g_of_row == g, qg, qh)
        qs.append(qh.astype(bf16))

    issue_until_pair(p_k + UPG - 1 + LAG)

    scale = DH ** -0.5
    nt = (((1,), (1,)), ((), ()))
    even_g = lax.broadcasted_iota(jnp.int32, (8, G), 0) % 2 == 0
    ms, ls, accs = [None] * HKV, [None] * HKV, [None] * HKV

    for j in range(NG):
        base = j * G
        wait_all(kbuf.at[:, pl.ds(base, G), :], S_K + j)
        wait_all(vbuf.at[:, pl.ds(base, G), :], S_V + j)
        if j < NG - 1:
            issue_until_pair(p_k + (j + 2) * UPG - 1 + LAG)
        else:
            issue_until_pair(p_k + NG * UPG - 1 + LAG + EXTRA)
            wait_all(w1_buf, S_W1)
            c_b1.wait()
        ss = []
        for h in range(HKV):
            s0 = lax.dot_general(qs[h], kbuf[h, pl.ds(base, G), :], nt, preferred_element_type=f32)
            s1 = lax.dot_general(qs[h], kbuf[HKV + h, pl.ds(base, G), :], nt, preferred_element_type=f32)
            ss.append(jnp.where(even_g, s0, s1) * scale)
        pbs, alphas = [], []
        for h in range(HKV):
            s = ss[h]
            m_cur = jnp.max(s, axis=-1, keepdims=True)
            m_new = m_cur if j == 0 else jnp.maximum(ms[h], m_cur)
            p = jnp.exp(s - m_new)
            psum = p[:, 0:DH]
            for t in range(1, G // DH):
                psum = psum + p[:, t * DH:(t + 1) * DH]
            if j == 0:
                alphas.append(None)
                ls[h] = psum
            else:
                alpha = jnp.exp(ms[h] - m_new)
                alphas.append(alpha)
                ls[h] = ls[h] * alpha + psum
            pbs.append(p.astype(bf16))
            ms[h] = m_new
        for h in range(HKV):
            o0 = jnp.dot(pbs[h], vbuf[h, pl.ds(base, G), :], preferred_element_type=f32)
            o1 = jnp.dot(pbs[h], vbuf[HKV + h, pl.ds(base, G), :], preferred_element_type=f32)
            o = jnp.where(even, o0, o1)
            accs[h] = o if j == 0 else accs[h] * alphas[h] + o

    heads = []
    for h in range(HKV):
        oh = accs[h] / jnp.sum(ls[h], axis=-1, keepdims=True)
        for g in range(REP):
            heads.append(oh if g == 0 else pltpu.roll(oh, 8 - 2 * g, 0))
    lhs = [o.astype(bf16) for o in heads]
    rolled = [pltpu.roll(o, 8, 1) for o in heads]
    lhs_prev = [jnp.where(lane128 < 8, rolled[i - 1], rolled[i]).astype(bf16) for i in range(HQ)]

    def coef(v, b):
        return jnp.transpose(jnp.broadcast_to(v.astype(f32)[b:b + 1], (DH, DH)))
    c_same = {seg: [coef(lhs[seg * REP + 3], b) for b in range(B)] for seg in (6, 7)}
    c_prev = {seg: [coef(lhs_prev[seg * REP + 3], b) for b in range(B)] for seg in (6, 7)}

    b1v = b1_buf[...].astype(f32)
    w1_cols = _col_tiles(w1_buf[...], F // 128)
    hdn = jnp.concatenate(
        [jnp.dot(xn, w1_cols[c], preferred_element_type=f32)
         + jnp.broadcast_to(b1v[c:c + 1], (8, DH)) for c in range(F // 128)], axis=1)
    sp = jnp.log1p(jnp.exp(-jnp.abs(hdn))) + jnp.maximum(hdn, 0.0)
    act = (hdn * jnp.tanh(sp)).astype(bf16)

    NC = D // 128
    outs = [x8[:, c * 128:(c + 1) * 128] for c in range(NC)]

    def add_wo(gi):
        for seg, g in wo_groups[gi]:
            i = seg * REP + g
            cols = _col_tiles(wo_buf[seg, g], NC)
            for cv in range(NC):
                c = (cv - O_WO) % NC
                a = lhs[i] if cv >= O_WO else lhs_prev[i]
                outs[c] = outs[c] + jnp.dot(a, cols[cv], preferred_element_type=f32)

    wait_all(w2_buf, S_W2)
    issue_until_pair(None)
    for gi in wo_first:
        wait_wo(gi)
    w2_cols = _col_tiles(w2_buf[...], NC)
    for c in range(NC):
        outs[c] = outs[c] + jnp.dot(act, w2_cols[c], preferred_element_type=f32)
    for gi in wo_first:
        add_wo(gi)

    for region in wo_regions:
        for gi in region:
            wait_wo(gi)
        for gi in region:
            add_wo(gi)

    vacc = [[None] * NC for _ in range(B)]
    for region in V_REGIONS:
        for vi in region:
            seg, a0, a1 = V_SLICES[vi]
            wait_all(wo_buf.at[seg, 3, pl.ds(NC * a0, NC * (a1 - a0))], S_LAST + vi)
        for vi in region:
            seg, a0, a1 = V_SLICES[vi]
            val = wo_buf[seg, 3, pl.ds(NC * a0, NC * (a1 - a0))].astype(f32)
            for a in range(a0, a1):
                for cv in range(NC):
                    c = (cv - O_WO) % NC
                    for b in range(B):
                        if cv >= O_WO:
                            cf = c_same[seg][b][8 * a:8 * a + 8]
                        elif a > 0:
                            cf = c_same[seg][b][8 * a - 8:8 * a]
                        else:
                            cf = c_prev[seg][b][0:8]
                        t = val[NC * (a - a0) + cv] * cf
                        vacc[b][c] = t if vacc[b][c] is None else vacc[b][c] + t
    res = []
    for c in range(NC):
        s0 = jnp.sum(vacc[0][c], axis=0, keepdims=True)
        s1 = jnp.sum(vacc[1][c], axis=0, keepdims=True)
        res.append(outs[c] + jnp.where(even, s0, s1))
    o_ref[...] = jnp.concatenate(res, axis=1)[0:B].astype(o_ref.dtype)


@jax.jit
def pallas_parallel_sum__sliding_block_cached__dense_activation_mish__decode_kernel(
    A_x: jax.Array,
    A_k_cache: jax.Array,
    A_v_cache: jax.Array,
    A_wq: jax.Array,
    A_wo: jax.Array,
    B_x: jax.Array,
    B_w1: jax.Array,
    B_b1: jax.Array,
    B_w2: jax.Array,
):
    del B_x
    SK = A_k_cache.shape[2]
    W = min(4096, max(256, SK // 4))
    assert A_x.shape == (B, 1, D) and A_k_cache.shape == (B, HKV, SK, DH) and W % G == 0
    assert A_wq.shape == (D, HQ * DH) and A_wo.shape == (HQ * DH, D)
    assert B_w1.shape == (D, F) and B_w2.shape == (F, D)
    bf16 = jnp.bfloat16
    x = A_x.reshape(B, D)
    b1 = B_b1.reshape(F // 128, 128)
    k = A_k_cache.reshape(NBH, SK, DH)
    v = A_v_cache.reshape(NBH, SK, DH)
    wq, wo, w1, w2 = _tiles(A_wq), _tiles(A_wo), _tiles(B_w1), _tiles(B_w2)
    n_sems = 5 + 2 * (W // G) + N_WO_GROUPS + len(V_SLICES)
    out = pl.pallas_call(
        functools.partial(_kernel, W=W, SK=SK),
        out_shape=jax.ShapeDtypeStruct((B, D), A_x.dtype),
        in_specs=[pl.BlockSpec(memory_space=pl.ANY)] * 8,
        out_specs=pl.BlockSpec(memory_space=pltpu.VMEM),
        scratch_shapes=[
            pltpu.VMEM((B, D), bf16),
            pltpu.VMEM((F // 128, 128), bf16),
            pltpu.VMEM((NBH, W, DH), bf16),
            pltpu.VMEM((NBH, W, DH), bf16),
            pltpu.VMEM(wq.shape, bf16),
            pltpu.VMEM((HKV, REP, 64, 8, 128), bf16),
            pltpu.VMEM(w1.shape, bf16),
            pltpu.VMEM(w2.shape, bf16),
            pltpu.SemaphoreType.DMA((n_sems,)),
        ],
        compiler_params=pltpu.CompilerParams(
            vmem_limit_bytes=100 * 1024 * 1024,
            disable_semaphore_checks=True,
        ),
    )(x, k, v, wq, wo, w1, b1, w2)
    return out.reshape(A_x.shape)
```

```python
import functools

import jax
import jax.numpy as jnp
from jax import lax
import jax.experimental.pallas as pl
import jax.experimental.pallas.tpu as pltpu

B, D = 2, 512
HQ, HKV, DH = 32, 8, 128
REP = HQ // HKV
F = 1792
NBH = B * HKV
CK = 128
G = 512
UT = 16
STEP = 16

KV_SHIFT = 16
O_WQ, O_WO, O_W1, O_W2 = 2, 2, 1, 15

LEAD = 24
LAG = 30
EXTRA = 14
N_WO_GROUPS = 9
V_SLICES = ((6, 0, 14), (6, 14, 16), (7, 0, 6), (7, 6, 10), (7, 10, 13), (7, 13, 16))
V_REGIONS = ((0,), (1, 2), (3,), (4,), (5,))


def _cyc(n, step):
    return [i for s in range(step) for i in range(s, n, step)]


def _tiles(w):
    r, c = w.shape
    return (w.reshape(r // 8, 8, c // 128, 128).transpose(0, 2, 1, 3)
            .reshape((r // 8) * (c // 128), 8, 128))


def _col_tiles(val, n_col_tiles):
    n = val.shape[0] // n_col_tiles
    v4 = val.reshape(n, n_col_tiles, 8, 128)
    return [v4[:, c].reshape(n * 8, 128) for c in range(n_col_tiles)]


def _kernel(x_hbm, k_hbm, v_hbm, wq_hbm, wo_hbm, w1_hbm, b1_hbm, w2_hbm, o_ref,
            x_buf, b1_buf, kbuf, vbuf, wq_buf, wo_buf, w1_buf, w2_buf, sems, *, W, SK):
    f32, bf16 = jnp.float32, jnp.bfloat16
    NG = W // G
    UPG = (G // CK) * NBH
    S_X, S_B1, S_WQ, S_W1, S_W2, S_K = 0, 1, 2, 3, 4, 5
    S_V = S_K + NG
    S_WO = S_V + NG
    S_LAST = S_WO + N_WO_GROUPS

    def cp(src, dst, si):
        return pltpu.make_async_copy(src, dst, sems.at[si]), si

    def w_units(src, dst, si, o):
        n = src.shape[0]

        def piece(a, m):
            return cp(src.at[pl.ds(a, m)], dst.at[pl.ds(a, m)], si)

        def unit(u):
            if u == 0:
                return [piece(0, UT - o), piece(n - o, o)]
            return [piece(UT * u - o, UT)]
        return [unit(u) for u in _cyc(n // UT, STEP)]

    def kv_unit(src, dst, si, j, c, r):
        off, sh, sem = j * G + c * CK, KV_SHIFT, si + j
        if off == 0:
            return [cp(src.at[r, pl.ds(SK - W, CK - sh), :], dst.at[r, pl.ds(sh, CK - sh), :], sem),
                    cp(src.at[r, pl.ds(SK - sh, sh), :], dst.at[r, pl.ds(0, sh), :], sem)]
        return [cp(src.at[r, pl.ds(SK - W + off - sh, CK), :], dst.at[r, pl.ds(off, CK), :], sem)]

    def wo_unit(seg, g, t0, nt, si):
        a, sem = (seg * REP + g) * 64 + t0 - O_WO, si
        if a < 0:
            return [cp(wo_hbm.at[pl.ds(0, nt + a)], wo_buf.at[seg, g, pl.ds(t0 - a, nt + a)], sem),
                    cp(wo_hbm.at[pl.ds(wo_hbm.shape[0] + a, -a)], wo_buf.at[seg, g, pl.ds(t0, -a)], sem)]
        return [cp(wo_hbm.at[pl.ds(a, nt)], wo_buf.at[seg, g, pl.ds(t0, nt)], sem)]

    hi = w_units(wq_hbm, wq_buf, S_WQ, O_WQ)
    lo = []
    p_k = len(hi)
    for j in range(NG):
        chunks = list(range(G // CK))
        if j == 0:
            chunks = chunks[1:] + chunks[:1]
        for c in chunks:
            for r in range(NBH):
                hi.append(kv_unit(k_hbm, kbuf, S_K, j, c, r))
                lo.append(kv_unit(v_hbm, vbuf, S_V, j, c, r))
    lo += w_units(w1_hbm, w1_buf, S_W1, O_W1)
    lo += w_units(w2_hbm, w2_buf, S_W2, O_W2)

    wo_groups = []

    def add_cycle(stream, blocks):
        si = S_WO + len(wo_groups)
        wo_groups.append(blocks)
        for c in range(64 // UT):
            for seg, g in blocks:
                stream.append(wo_unit(seg, g, c * UT, UT, si))

    add_cycle(hi, [(s, 0) for s in range(4)])
    add_cycle(hi, [(s, 1) for s in range(4)])
    add_cycle(hi, [(s, 2) for s in range(4)])
    add_cycle(hi, [(0, 3)])
    add_cycle(lo, [(1, 3), (2, 3), (3, 3)])
    add_cycle(lo, [(s, 0) for s in range(4, 8)])
    add_cycle(lo, [(s, 1) for s in range(4, 8)])
    add_cycle(lo, [(s, 2) for s in range(4, 8)])
    add_cycle(lo, [(4, 3), (5, 3)])
    for vi, (seg, a0, a1) in enumerate(V_SLICES):
        lo += [wo_unit(seg, 3, 4 * a, 4, S_LAST + vi) for a in range(a0, a1)]
    assert len(wo_groups) == N_WO_GROUPS
    wo_first = [0, 4, 5]
    wo_regions = [[1, 6], [2, 7], [3, 8]]

    seq = [(c, 1) for u in lo[:LEAD] for c in u]
    seq[1:1] = [(cp(x_hbm, x_buf, S_X), 0), (cp(b1_hbm, b1_buf, S_B1), 0)]
    pos_of_pair = []
    rest = lo[LEAD:]
    for i in range(max(len(hi), len(rest))):
        if i < len(hi):
            seq += [(c, 0) for c in hi[i]]
        if i < len(rest):
            seq += [(c, 1) for c in rest[i]]
        pos_of_pair.append(len(seq))
    issued = [0]

    def issue_until_pair(p):
        end = len(seq) if p is None or p >= len(pos_of_pair) else pos_of_pair[p]
        for (c, _), pr in seq[issued[0]:end]:
            c.start(priority=pr)
        issued[0] = max(issued[0], end)

    def wait_all(ref, si):
        assert all(s != si for (_, s), _ in seq[issued[0]:]), "waiting on copies not started yet"
        pltpu.make_async_copy(ref, ref, sems.at[si]).wait()

    def wait_wo(gi):
        blocks = wo_groups[gi]
        wait_all(wo_buf.at[pl.ds(blocks[0][0], len(blocks)), blocks[0][1]], S_WO + gi)

    issue_until_pair(p_k - 1 + LAG)

    wait_all(x_buf, S_X)
    row = lax.broadcasted_iota(jnp.int32, (8, D), 0)
    x2 = x_buf[...].astype(f32)
    x8 = jnp.where(row % 2 == 0, jnp.broadcast_to(x2[0:1], (8, D)), jnp.broadcast_to(x2[1:2], (8, D)))
    mu = jnp.mean(x8, axis=-1, keepdims=True)
    xc = x8 - mu
    var = jnp.mean(xc * xc, axis=-1, keepdims=True)
    xn = (xc / jnp.sqrt(var + 1e-5)).astype(bf16)

    row128 = lax.broadcasted_iota(jnp.int32, (8, DH), 0)
    lane128 = lax.broadcasted_iota(jnp.int32, (8, DH), 1)
    g_of_row = row128 // 2
    even = row128 % 2 == 0

    wait_all(wq_buf, S_WQ)
    wq_cols = _col_tiles(wq_buf[...], HQ)
    qs = []
    for h in range(HKV):
        qh = None
        for g in range(REP):
            qg = jnp.dot(xn, wq_cols[h * REP + g], preferred_element_type=f32)
            qh = qg if g == 0 else jnp.where(g_of_row == g, qg, qh)
        qs.append(qh.astype(bf16))

    issue_until_pair(p_k + UPG - 1 + LAG)

    scale = DH ** -0.5
    nt = (((1,), (1,)), ((), ()))
    even_g = lax.broadcasted_iota(jnp.int32, (8, G), 0) % 2 == 0
    ms, ls, accs = [None] * HKV, [None] * HKV, [None] * HKV

    for j in range(NG):
        base = j * G
        wait_all(kbuf.at[:, pl.ds(base, G), :], S_K + j)
        wait_all(vbuf.at[:, pl.ds(base, G), :], S_V + j)
        if j < NG - 1:
            issue_until_pair(p_k + (j + 2) * UPG - 1 + LAG)
        else:
            issue_until_pair(p_k + NG * UPG - 1 + LAG + EXTRA)
            wait_all(w1_buf, S_W1)
            wait_all(b1_buf, S_B1)
        ss = []
        for h in range(HKV):
            s0 = lax.dot_general(qs[h], kbuf[h, pl.ds(base, G), :], nt, preferred_element_type=f32)
            s1 = lax.dot_general(qs[h], kbuf[HKV + h, pl.ds(base, G), :], nt, preferred_element_type=f32)
            ss.append(jnp.where(even_g, s0, s1) * scale)
        pbs, alphas = [], []
        for h in range(HKV):
            s = ss[h]
            m_cur = jnp.max(s, axis=-1, keepdims=True)
            m_new = m_cur if j == 0 else jnp.maximum(ms[h], m_cur)
            p = jnp.exp(s - m_new)
            psum = p[:, 0:DH]
            for t in range(1, G // DH):
                psum = psum + p[:, t * DH:(t + 1) * DH]
            if j == 0:
                alphas.append(None)
                ls[h] = psum
            else:
                alpha = jnp.exp(ms[h] - m_new)
                alphas.append(alpha)
                ls[h] = ls[h] * alpha + psum
            pbs.append(p.astype(bf16))
            ms[h] = m_new
        for h in range(HKV):
            o0 = jnp.dot(pbs[h], vbuf[h, pl.ds(base, G), :], preferred_element_type=f32)
            o1 = jnp.dot(pbs[h], vbuf[HKV + h, pl.ds(base, G), :], preferred_element_type=f32)
            o = jnp.where(even, o0, o1)
            accs[h] = o if j == 0 else accs[h] * alphas[h] + o

    heads = []
    for h in range(HKV):
        oh = accs[h] / jnp.sum(ls[h], axis=-1, keepdims=True)
        for g in range(REP):
            heads.append(oh if g == 0 else pltpu.roll(oh, 8 - 2 * g, 0))
    lhs = [o.astype(bf16) for o in heads]
    rolled = [pltpu.roll(o, 8, 1) for o in heads]
    lhs_prev = [jnp.where(lane128 < 8, rolled[i - 1], rolled[i]).astype(bf16) for i in range(HQ)]

    def coef(v, b):
        return jnp.transpose(jnp.broadcast_to(v.astype(f32)[b:b + 1], (DH, DH)))
    c_same = {seg: [coef(lhs[seg * REP + 3], b) for b in range(B)] for seg in (6, 7)}
    c_prev = {seg: [coef(lhs_prev[seg * REP + 3], b) for b in range(B)] for seg in (6, 7)}

    b1v = b1_buf[...].astype(f32)
    w1_cols = _col_tiles(w1_buf[...], F // 128)
    hdn = jnp.concatenate(
        [jnp.dot(xn, w1_cols[c], preferred_element_type=f32)
         + jnp.broadcast_to(b1v[c:c + 1], (8, DH)) for c in range(F // 128)], axis=1)
    sp = jnp.log1p(jnp.exp(-jnp.abs(hdn))) + jnp.maximum(hdn, 0.0)
    act = (hdn * jnp.tanh(sp)).astype(bf16)

    NC = D // 128
    outs = [x8[:, c * 128:(c + 1) * 128] for c in range(NC)]

    def add_wo(gi):
        for seg, g in wo_groups[gi]:
            i = seg * REP + g
            cols = _col_tiles(wo_buf[seg, g], NC)
            for cv in range(NC):
                c = (cv - O_WO) % NC
                a = lhs[i] if cv >= O_WO else lhs_prev[i]
                outs[c] = outs[c] + jnp.dot(a, cols[cv], preferred_element_type=f32)

    wait_all(w2_buf, S_W2)
    issue_until_pair(None)
    for gi in wo_first:
        wait_wo(gi)
    w2_cols = _col_tiles(w2_buf[...], NC)
    for c in range(NC):
        outs[c] = outs[c] + jnp.dot(act, w2_cols[c], preferred_element_type=f32)
    for gi in wo_first:
        add_wo(gi)

    for region in wo_regions:
        for gi in region:
            wait_wo(gi)
        for gi in region:
            add_wo(gi)

    vacc = [[None] * NC for _ in range(B)]
    for region in V_REGIONS:
        for vi in region:
            seg, a0, a1 = V_SLICES[vi]
            wait_all(wo_buf.at[seg, 3, pl.ds(NC * a0, NC * (a1 - a0))], S_LAST + vi)
        for vi in region:
            seg, a0, a1 = V_SLICES[vi]
            val = wo_buf[seg, 3, pl.ds(NC * a0, NC * (a1 - a0))].astype(f32)
            for a in range(a0, a1):
                for cv in range(NC):
                    c = (cv - O_WO) % NC
                    for b in range(B):
                        if cv >= O_WO:
                            cf = c_same[seg][b][8 * a:8 * a + 8]
                        elif a > 0:
                            cf = c_same[seg][b][8 * a - 8:8 * a]
                        else:
                            cf = c_prev[seg][b][0:8]
                        t = val[NC * (a - a0) + cv] * cf
                        vacc[b][c] = t if vacc[b][c] is None else vacc[b][c] + t
    res = []
    for c in range(NC):
        s0 = jnp.sum(vacc[0][c], axis=0, keepdims=True)
        s1 = jnp.sum(vacc[1][c], axis=0, keepdims=True)
        res.append(outs[c] + jnp.where(even, s0, s1))
    o_ref[...] = jnp.concatenate(res, axis=1)[0:B].astype(o_ref.dtype)


@jax.jit
def pallas_parallel_sum__sliding_block_cached__dense_activation_mish__decode_kernel(
    A_x: jax.Array,
    A_k_cache: jax.Array,
    A_v_cache: jax.Array,
    A_wq: jax.Array,
    A_wo: jax.Array,
    B_x: jax.Array,
    B_w1: jax.Array,
    B_b1: jax.Array,
    B_w2: jax.Array,
):
    del B_x
    SK = A_k_cache.shape[2]
    W = min(4096, max(256, SK // 4))
    assert A_x.shape == (B, 1, D) and A_k_cache.shape == (B, HKV, SK, DH) and W % G == 0
    assert A_wq.shape == (D, HQ * DH) and A_wo.shape == (HQ * DH, D)
    assert B_w1.shape == (D, F) and B_w2.shape == (F, D)
    bf16 = jnp.bfloat16
    x = A_x.reshape(B, D)
    b1 = B_b1.reshape(F // 128, 128)
    k = A_k_cache.reshape(NBH, SK, DH)
    v = A_v_cache.reshape(NBH, SK, DH)
    wq, wo, w1, w2 = _tiles(A_wq), _tiles(A_wo), _tiles(B_w1), _tiles(B_w2)
    n_sems = 5 + 2 * (W // G) + N_WO_GROUPS + len(V_SLICES)
    out = pl.pallas_call(
        functools.partial(_kernel, W=W, SK=SK),
        out_shape=jax.ShapeDtypeStruct((B, D), A_x.dtype),
        in_specs=[pl.BlockSpec(memory_space=pl.ANY)] * 8,
        out_specs=pl.BlockSpec(memory_space=pltpu.VMEM),
        scratch_shapes=[
            pltpu.VMEM((B, D), bf16),
            pltpu.VMEM((F // 128, 128), bf16),
            pltpu.VMEM((NBH, W, DH), bf16),
            pltpu.VMEM((NBH, W, DH), bf16),
            pltpu.VMEM(wq.shape, bf16),
            pltpu.VMEM((HKV, REP, 64, 8, 128), bf16),
            pltpu.VMEM(w1.shape, bf16),
            pltpu.VMEM(w2.shape, bf16),
            pltpu.SemaphoreType.DMA((n_sems,)),
        ],
        compiler_params=pltpu.CompilerParams(
            vmem_limit_bytes=100 * 1024 * 1024,
            disable_semaphore_checks=True,
        ),
    )(x, k, v, wq, wo, w1, b1, w2)
    return out.reshape(A_x.shape)
```
